```python
import os as _os
_os.environ.setdefault("JAX_PLATFORMS", "cpu")
import jax
import jax.numpy as jnp

def _softmax(x, axis=-1):
    return jax.nn.softmax(x, axis=axis)
def _gelu(x):
    return jax.nn.gelu(x, approximate=True)
def _silu(x):
    return jax.nn.silu(x)
def _sigmoid(x):
    return jax.nn.sigmoid(x)
def _layernorm(x, axis=-1, eps=1e-5):
    m = jnp.mean(x, axis=axis, keepdims=True)
    v = jnp.var(x, axis=axis, keepdims=True)
    return (x - m) / jnp.sqrt(v + eps)
def _scatter_add(tgt, idx, src, axis=0):
    return tgt.at[idx].add(src)
def _segment_sum(src, seg, n):
    return jax.ops.segment_sum(src, seg, n)
class _Rng:
    def __init__(self, key):
        self._k = key
    def _next(self):
        self._k, sub = jax.random.split(self._k)
        return sub
    def normal(self, shape):
        return jax.random.normal(self._next(), shape, dtype=jnp.bfloat16)
    def randint(self, lo, hi, shape):
        return jax.random.randint(self._next(), shape, lo, hi, dtype=jnp.int32)
    def uniform(self, shape, lo=0.0, hi=1.0):
        return jax.random.uniform(self._next(), shape, jnp.bfloat16, lo, hi)
    def permutation(self, n):
        return jax.random.permutation(self._next(), n)


kernel_name = 'concat_heads__mha_block__linear_attn_block__prompt'

def setup_inputs():
    _rng = _Rng(jax.random.key(int.from_bytes(__import__("os").urandom(4), "little")))
    _w = (lambda a: (lambda t: t.astype(jnp.bfloat16) if jnp.issubdtype(t.dtype, jnp.floating) else t)(jnp.asarray(a)))
    def _A_setup():
        B, S, D, H = 1, 2048, 1024, 32
        return {
            "x": _w((lambda *s: _rng.normal(s) * 0.2)(B, S, D)),
            "wqkv": _w((lambda *s: _rng.normal(s) * 0.2)(D, 3 * D)),
            "wo": _w((lambda *s: _rng.normal(s) * 0.05)(D, D)),
        }
    _A_in = _A_setup()

    def _B_setup():
        B, S, D = 1, 2048, 1024
        return {
            "x": _w((lambda *s: _rng.normal(s) * 0.05)(B, S, D)),
            "wqkv": _w((lambda *s: _rng.normal(s) * 1.6)(D, 3 * D)),
            "wo": _w((lambda *s: _rng.normal(s) * 0.1)(D, D)),
        }
    _B_in = _B_setup()

    return {
        "A_x": _A_in["x"],
        "A_wqkv": _A_in["wqkv"],
        "A_wo": _A_in["wo"],
        "B_x": _B_in["x"],
        "B_wqkv": _B_in["wqkv"],
        "B_wo": _B_in["wo"],
    }

def reference(A_x, A_wqkv, A_wo, B_x, B_wqkv, B_wo):
    def _A_ref(x, wqkv, wo):
        B, S, D = x.shape
        H = 32
        Dh = D // H
        qkv = (lambda x, *d: x.transpose(*d))((x @ wqkv).reshape(B, S, 3, H, Dh), 2, 0, 3, 1, 4)
        q, k, v = qkv[0], qkv[1], qkv[2]
        scores = jnp.einsum("bhqd,bhkd->bhqk", q, k) * (Dh ** -0.5)
        p = _softmax(scores, axis=-1)
        o = jnp.einsum("bhqk,bhkd->bhqd", p, v)
        return (lambda x, *d: x.transpose(*d))(o, 0, 2, 1, 3).reshape(B, S, D) @ wo

    def _B_ref(x, wqkv, wo):
        B, S, D = x.shape
        H = 32; Dh = D // H
        qkv = (lambda x, *d: x.transpose(*d))((x @ wqkv).reshape(B, S, 3, H, Dh), 2, 0, 3, 1, 4)
        q, k, v = qkv[0], qkv[1], qkv[2]
        phi = lambda t: jnp.where(t > 0, t + 1, jnp.exp(t)) + 1e-6
        pq, pk = phi(q), phi(k)
        kv = jnp.einsum("bhsd,bhse->bhde", pk, v)
        z = jnp.einsum("bhsd->bhd", pk)
        num = jnp.einsum("bhqd,bhde->bhqe", pq, kv)
        den = jnp.einsum("bhqd,bhd->bhq", pq, z)[..., None] + 1e-6
        o = num / den
        return (lambda x, *d: x.transpose(*d))(o, 0, 2, 1, 3).reshape(B, S, D) @ wo

    a = _A_ref(A_x, A_wqkv, A_wo)
    b = _B_ref(B_x, B_wqkv, B_wo)
    return jnp.concatenate([a, b], axis=-1)
```

```python
import math
import jax
import jax.numpy as jnp
from jax import lax
import jax.experimental.pallas as pl
import jax.experimental.pallas.tpu as pltpu

S, D, H, DH = 2048, 1024, 32, 32
G = D // 128
RB = 512
NRB = S // RB
TQ = 512
TK = 256
NQ = S // TQ
NK = S // TK
NU = H * NQ
QSCALE = (DH ** -0.5) * math.log2(math.e)
NT = (((1,), (1,)), ((), ()))
TN = (((0,), (0,)), ((), ()))
BF = jnp.bfloat16
F32 = jnp.float32


def _phi(t):
    return jnp.where(t > 0, t + 1.0, jnp.exp(t)) + 1e-6


def _kernel(xa_h, wa_h, woa_h, xb_h, wb_h, wob_h, out_h,
            xa, wa, woa, xb, wb, wob,
            qt, kk, vt, pk, vtb, kvz, zacc, sbuf, ot, obuf,
            sem_in, sem_out):
    copies = {}

    def cp(name, src, dst, i):
        c = pltpu.make_async_copy(src, dst, sem_in.at[i])
        c.start()
        copies[name] = c

    n = 0
    cp(('xa', 0), xa_h.at[0, pl.ds(0, RB)], xa.at[pl.ds(0, RB)], n); n += 1
    cp(('wa', 0), wa_h.at[:, pl.ds(0, D)], wa.at[0], n); n += 1
    for r in range(1, NRB):
        cp(('xa', r), xa_h.at[0, pl.ds(r * RB, RB)], xa.at[pl.ds(r * RB, RB)], n); n += 1
    cp(('wa', 2), wa_h.at[:, pl.ds(2 * D, D)], wa.at[2], n); n += 1
    cp(('wa', 1), wa_h.at[:, pl.ds(D, D)], wa.at[1], n); n += 1
    cp('xb', xb_h.at[0], xb, n); n += 1
    for c in (1, 2, 0):
        cp(('wb', c), wb_h.at[:, pl.ds(c * D, D)], wb.at[c], n); n += 1
    cp('wob', wob_h, wob, n); n += 1
    cp('woa', woa_h, woa, n); n += 1

    def out_copy(slot, r, col):
        return pltpu.make_async_copy(
            obuf.at[slot], out_h.at[0, pl.ds(r * RB, RB), pl.ds(col, D)], sem_out.at[slot])

    def proj_t(x_ref, w, dst, r, scale):
        rows = pl.ds(pl.multiple_of(r * RB, RB), RB)
        y = jnp.dot(x_ref[rows, :], w, preferred_element_type=F32)
        if scale is not None:
            y = y * scale
        for t in range(RB // 128):
            dst[r * (RB // 128) + t] = y[t * 128:(t + 1) * 128, :].T.astype(BF)

    copies[('wa', 0)].wait()
    for r in range(NRB):
        copies[('xa', r)].wait()
        proj_t(xa, wa[0], qt, r, QSCALE)
    copies[('wa', 2)].wait()
    lax.fori_loop(0, NRB, lambda r, c: (proj_t(xa, wa[2], vt, r, None), c)[1], 0)
    copies[('wa', 1)].wait()

    def ka_body(r, c):
        rows = pl.ds(pl.multiple_of(r * RB, RB), RB)
        y = jnp.dot(xa[rows, :], wa[1], preferred_element_type=F32).astype(BF)
        for g in range(G):
            kk[g, rows, :] = y[:, g * 128:(g + 1) * 128]
        return c
    lax.fori_loop(0, NRB, ka_body, 0)

    copies['xb'].wait()
    copies[('wb', 1)].wait()
    zacc[...] = jnp.zeros_like(zacc)

    def kb_body(r, c):
        rows = pl.ds(pl.multiple_of(r * RB, RB), RB)
        y = _phi(jnp.dot(xb[rows, :], wb[1], preferred_element_type=F32))
        zacc[...] += y.reshape(RB // 8, 8, D).sum(axis=0)
        y = y.astype(BF)
        for g in range(G):
            pk[g, rows, :] = y[:, g * 128:(g + 1) * 128]
        return c
    lax.fori_loop(0, NRB, kb_body, 0)
    copies[('wb', 2)].wait()
    lax.fori_loop(0, NRB, lambda r, c: (proj_t(xb, wb[2], vtb, r, None), c)[1], 0)

    rr = lax.broadcasted_iota(jnp.int32, (128, 128), 0) // DH
    cc = lax.broadcasted_iota(jnp.int32, (128, 128), 1) // DH
    bd = rr == cc
    z = jnp.sum(zacc[...], axis=0, keepdims=True)
    for g in range(G):
        vg = jnp.concatenate([vtb[t, g * 128:(g + 1) * 128, :] for t in range(S // 128)], axis=1)
        kvt = jnp.dot(vg, pk[g], preferred_element_type=F32)
        kvz[g, 0:128, :] = jnp.where(bd, kvt, 0.0).astype(BF)
        kvz[g, 128:256, :] = jnp.where(bd, z[:, g * 128:(g + 1) * 128], 0.0).astype(BF)

    copies[('wb', 0)].wait()
    copies['wob'].wait()

    def qb_body(r, c):
        rows = pl.ds(pl.multiple_of(r * RB, RB), RB)
        pq = _phi(jnp.dot(xb[rows, :], wb[0], preferred_element_type=F32)).astype(BF)
        os_ = []
        for g in range(G):
            nd = lax.dot_general(pq[:, g * 128:(g + 1) * 128], kvz[g], NT, preferred_element_type=F32)
            os_.append((nd[:, :128] / (nd[:, 128:] + 1e-6)).astype(BF))
        o = jnp.concatenate(os_, axis=1)
        obuf[NRB + r] = jnp.dot(o, wob[...], preferred_element_type=F32).astype(BF)
        out_copy(NRB + r, r, D).start()
        return c
    lax.fori_loop(0, NRB, qb_body, 0)

    copies['woa'].wait()
    rowgrp = lax.broadcasted_iota(jnp.int32, (128, TQ), 0) // DH

    def step(u1, u2, m_prev):
        if u1 is not None:
            qi, h = u1 // H, u1 % H
            g = h // 4
            hrow = pl.ds(pl.multiple_of(h * DH, DH), DH)
            qh = jnp.concatenate([qt[qi * (TQ // 128) + t, hrow, :] for t in range(TQ // 128)], axis=1)
            wq = jnp.where(rowgrp == h % 4, jnp.concatenate([qh] * 4, axis=0), jnp.zeros((), BF))
        if u2 is not None:
            h2 = u2 % H
            hrow2 = pl.ds(pl.multiple_of(h2 * DH, DH), DH)
        m8 = l8 = acc = None
        for c in range(NK):
            rows = slice(c * TK, (c + 1) * TK)
            if u1 is not None:
                st = jnp.dot(kk[g, rows, :], wq, preferred_element_type=F32)
            if u2 is not None:
                p = jnp.exp2(sbuf[rows, :] - m_prev)
                ls = p.reshape(TK // 8, 8, TQ).sum(axis=0)
                l8 = ls if l8 is None else l8 + ls
                pb = p.astype(BF)
            if u1 is not None:
                sbuf[rows, :] = st
                mc = st.reshape(TK // 8, 8, TQ).max(axis=0)
                m8 = mc if m8 is None else jnp.maximum(m8, mc)
            if u2 is not None:
                vh = jnp.concatenate([vt[c * (TK // 128) + t, hrow2, :] for t in range(TK // 128)], axis=1)
                o = jnp.dot(vh, pb, preferred_element_type=F32)
                acc = o if acc is None else o + acc
        if u2 is not None:
            l = jnp.sum(l8, axis=0, keepdims=True)
            ot[hrow2, :] = (acc / l).astype(BF)
        if u1 is not None:
            return jnp.max(m8, axis=0, keepdims=True)
        return None

    def out_proj(qi):
        obuf[qi] = lax.dot_general(ot[...], woa[...], TN, preferred_element_type=F32).astype(BF)
        out_copy(qi, qi, 0).start()

    m0 = step(0, None, None)

    def body(u, m):
        m = step(u, u - 1, m)

        @pl.when(u % H == 0)
        def _():
            out_proj(u // H - 1)
        return m
    m = lax.fori_loop(1, NU, body, m0)
    step(None, NU - 1, m)
    out_proj(NQ - 1)

    for r in range(NRB):
        out_copy(r, r, 0).wait()
        out_copy(NRB + r, r, D).wait()


@jax.jit
def pallas_concat_heads__mha_block__linear_attn_block__prompt_kernel(A_x, A_wqkv, A_wo, B_x, B_wqkv, B_wo):
    any_spec = pl.BlockSpec(memory_space=pl.ANY)
    return pl.pallas_call(
        _kernel,
        out_shape=jax.ShapeDtypeStruct((1, S, 2 * D), BF),
        in_specs=[any_spec] * 6,
        out_specs=any_spec,
        scratch_shapes=[
            pltpu.VMEM((S, D), BF), pltpu.VMEM((3, D, D), BF), pltpu.VMEM((D, D), BF),
            pltpu.VMEM((S, D), BF), pltpu.VMEM((3, D, D), BF), pltpu.VMEM((D, D), BF),
            pltpu.VMEM((S // 128, D, 128), BF),
            pltpu.VMEM((G, S, 128), BF),
            pltpu.VMEM((S // 128, D, 128), BF),
            pltpu.VMEM((G, S, 128), BF),
            pltpu.VMEM((S // 128, D, 128), BF),
            pltpu.VMEM((G, 256, 128), BF),
            pltpu.VMEM((8, D), F32),
            pltpu.VMEM((S, TQ), F32),
            pltpu.VMEM((D, TQ), BF),
            pltpu.VMEM((2 * NRB, RB, D), BF),
            pltpu.SemaphoreType.DMA((16,)),
            pltpu.SemaphoreType.DMA((2 * NRB,)),
        ],
        compiler_params=pltpu.CompilerParams(vmem_limit_bytes=110 * 1024 * 1024),
    )(A_x, A_wqkv, A_wo, B_x, B_wqkv, B_wo)
```

```python
import math
import jax
import jax.numpy as jnp
from jax import lax
import jax.experimental.pallas as pl
import jax.experimental.pallas.tpu as pltpu

S, D, H, DH = 2048, 1024, 32, 32
G = D // 128
TQ = 512
TK = 256
NQ = S // TQ
NK = S // TK
NT128 = S // 128
TPQ = TQ // 128
NB = NQ * G
HB = 256
NHB = S // HB
NU = 13
NU_EPI = 12
NU_0 = 9
MID = 27
QSCALE = (DH ** -0.5) * math.log2(math.e)
TN = (((0,), (0,)), ((), ()))
BF = jnp.bfloat16
F32 = jnp.float32
SCOPES = False

W_SRC = (0, 0, 0, 1, 1, 1, 2)
W_NAT = (0, 3, 3, 3, 1, 3, 2)
W_TT = (4, 0, 1, 2, 4, 3, 4)
W_ACT = (0, 1, 0, 2, 0, 2, 0)
SLOTS = [(0, 2), (0, 4), (0, 6), (1, 0), (1, 2), (1, 4), (1, 6), (2, 0), (2, 2), (2, 4), (2, 6), (3, 0), (3, 2)]
OSLOT = (0, 0)
EPI_FINE = 7
EPI_PRE = 1


def _schedule():
    a_units = [(w, r, g) for g in range(1, G) for w in (0, 1, 2) for r in range(NHB)]
    b_pre = [(w, r, c) for w in (3, 4, 5) for r in range(NHB) for c in range(G)]
    b_out = [(6, r, c) for r in range(NHB) for c in range(G)]
    quota_a = [9, 13] + [6] * 24 + [2, 0] + [0] * 4
    assert len(quota_a) == NB and sum(quota_a) == len(a_units)
    sched = []
    for i in range(NB):
        us = [a_units.pop(0) for _ in range(quota_a[i])]
        src = b_pre if i <= MID else b_out
        us += [src.pop(0) for _ in range((NU if i else NU_0) - quota_a[i])]
        sched.append(us)
        if i == MID:
            assert not b_pre
    assert len(b_out) == NU_EPI
    sched.append(b_out)
    done = set()
    for i in range(NB):
        done.update(sched[i])
        g = i // NQ + 1
        if g < G and i % NQ == 1:
            assert all((w, r, g) in done for w in (0, 1) for r in range(NHB)), i
        if g < G and i % NQ == 2:
            assert all((2, r, g) in done for r in range(NHB)), i
    return sched


SCHED = _schedule()


def _pack(u):
    w, r, c = u
    return (w | r << 3 | c << 6 | W_SRC[w] << 9 | W_NAT[w] << 11 | W_TT[w] << 13 | W_ACT[w] << 16
            | (0 if w == 3 else 1) << 18)


class _Null:
    def __enter__(self):
        return self

    def __exit__(self, *a):
        return False


def _scope(name):
    return jax.named_scope(name) if SCOPES else _Null()


def _phi(t):
    return jnp.where(t > 0, t + 1.0, jnp.exp(t)) + 1e-6


def _divmod_pow2(i, n):
    if isinstance(i, int):
        return i // n, i % n
    return lax.shift_right_logical(i, int(math.log2(n))), i & (n - 1)


def _ds(i, size):
    return pl.ds(i * size if isinstance(i, int) else pl.multiple_of(i * size, size), size)


def _kernel(xa_h, wa_h, woa_h, xb_h, wb_h, wob_h, out_h,
            x, w, nat, tt, cur, zacc, sbuf, mbuf, lbuf, oacc, acca, obufa, tab,
            sem_in, sem_out, sem_f):
    def w_src(wi, c):
        if wi < 3:
            return wa_h.at[:, pl.ds((1, 0, 2)[wi] * D + c * 128, 128)]
        if wi < 6:
            return wb_h.at[:, pl.ds((1, 2, 0)[wi - 3] * D + c * 128, 128)]
        return (wob_h, woa_h)[wi - 6].at[:, pl.ds(c * 128, 128)]

    def cw(pairs, s):
        return [pltpu.make_async_copy(w_src(wi, c), w.at[wi, c], sem_in.at[s]) for wi, c in pairs]

    def cxa(r):
        rows = pl.ds(r * TQ, TQ)
        return [pltpu.make_async_copy(xa_h.at[0, rows, pl.ds(k * 128, 128)], x.at[0, k, rows], sem_in.at[r])
                for k in range(G)]

    cxb = [pltpu.make_async_copy(xb_h.at[0, :, pl.ds(k * 128, 128)], x.at[1, k], sem_in.at[4]) for k in range(G)]
    cw0 = cw([(wi, 0) for wi in (1, 2, 0)], 5)
    cw1 = cw([(wi, c) for c in (1, 2) for wi in (0, 1, 2)], 6)
    cw2 = cw([(7, c) for c in range(G)], 7)
    cw3 = cw([(wi, c) for c in range(3, G) for wi in (0, 1, 2)] + [(3, c) for c in range(G)], 8)
    cw4 = cw([(wi, c) for wi in (4, 5, 6) for c in range(G)], 9)

    def start(cs):
        for c in cs:
            c.start()

    def wait(cs):
        for c in cs:
            c.wait()

    def out_copy_a(r):
        return pltpu.make_async_copy(
            obufa.at[r], out_h.at[0, _ds(r, TQ), pl.ds(0, D)], sem_out.at[r])

    def out_copy_b(n):
        r, c = _divmod_pow2(n, G)
        return pltpu.make_async_copy(
            nat.at[2, c, _ds(r, HB)], out_h.at[0, _ds(r, HB), _ds(G + c, 128)], sem_out.at[NQ])

    def f_out(k, g):
        src = nat.at[0, g] if k == 0 else tt.at[k - 1, g]
        return pltpu.make_async_copy(src, out_h.at[0, :, pl.ds(k * 128, 128)], sem_f.at[k])

    def f_in(k, g):
        return pltpu.make_async_copy(out_h.at[0, :, pl.ds(k * 128, 128)], cur.at[k, g & 1], sem_f.at[3 + k])

    def unit_mm(u, rh=None, kh=None):
        wi, r, c = u
        rows = _ds(r, HB) if rh is None else pl.ds(r * HB + rh * 128, 128)
        ks = range(G) if kh is None else range(kh * G // 2, (kh + 1) * G // 2)
        lhs = jnp.concatenate([x[W_SRC[wi], k, rows, :] for k in ks], axis=1)
        return jnp.dot(lhs, w[wi, c, ks[0] * 128:(ks[-1] + 1) * 128, :], preferred_element_type=F32)

    def unit(u, direct=False):
        static = isinstance(u, tuple)
        if static:
            wi, r, c = u
            src, ni, ti, act = W_SRC[wi], W_NAT[wi], W_TT[wi], W_ACT[wi]
            zi = 0 if wi == 3 else 1
        else:
            f = lambda sh, bits: lax.shift_right_logical(u, sh) & ((1 << bits) - 1)
            wi, r, c, src, ni, ti, act, zi = (f(0, 3), f(3, 3), f(6, 3), f(9, 2), f(11, 2), f(13, 3),
                                              f(16, 2), f(18, 1))
        rows = _ds(r, HB)
        lhs = jnp.concatenate([x[src, k, rows, :] for k in range(G)], axis=1)
        y = jnp.dot(lhs, w[wi, c], preferred_element_type=F32)
        if static:
            if act == 1:
                y = y * QSCALE
            elif act == 2:
                y = _phi(y)
        else:
            y = jnp.where(act == 2, _phi(y), y * jnp.where(act == 1, QSCALE, 1.0))
        y_t = jnp.concatenate([y[t * 128:(t + 1) * 128, :].T for t in range(HB // 128)], axis=0)
        if direct:
            cur[wi, 0, rows, :] = (y if wi == 0 else y_t).astype(BF)
            return
        if not static or zi == 0:
            zacc[zi, c] += y.reshape(HB // 8, 8, 128).sum(axis=0)
        if not static or ni != 3:
            nat[ni, c, rows, :] = y.astype(BF)
        if not static or ti != 4:
            tt[ti, c, rows, :] = y_t.astype(BF)

    start(cw0)
    start(cxa(0))
    zacc[...] = jnp.zeros_like(zacc)
    oacc[...] = jnp.zeros_like(oacc)
    lbuf[...] = jnp.ones_like(lbuf)
    for i in range(1, NB):
        for k, u in enumerate(SCHED[i]):
            tab[i * NU + k] = _pack(u)

    def up_body(r, c):
        @pl.when(r == 0)
        def _():
            wait(cw0)
            wait(cxa(0))
            for rr in range(1, NQ):
                start(cxa(rr))

        @pl.when(r == 1)
        def _():
            wait(cxa(1))
            start(cw1)

        @pl.when(r == 2)
        def _():
            wait(cxa(2))

        @pl.when(r == 3)
        def _():
            wait(cxa(3))
            start(cw2)
            start(cxb)
            start(cw3)
            start(cw4)

        for wi in (1, 2, 0):
            for hh in range(TQ // HB):
                unit((wi, r * (TQ // HB) + hh, 0), direct=True)
        return c
    with _scope('upfront'):
        lax.fori_loop(0, NQ, up_body, 0)

    def b_mid():
        rr = lax.broadcasted_iota(jnp.int32, (128, 128), 0) // DH
        cc = lax.broadcasted_iota(jnp.int32, (128, 128), 1) // DH
        bd = rr == cc
        zr = lax.broadcasted_iota(jnp.int32, (16, 128), 0)
        zc = lax.broadcasted_iota(jnp.int32, (16, 128), 1) // DH
        kvs = []

        def m_rows(g):
            gs = slice(g * 128, (g + 1) * 128)
            wo = jnp.concatenate([w[6, c, gs, :] for c in range(G)], axis=1)
            m = jnp.dot(kvs[g], wo, preferred_element_type=F32).astype(BF)
            for c in range(G):
                w[6, c, gs, :] = m[:, c * 128:(c + 1) * 128]

        for g in range(G):
            pkt = jnp.concatenate([tt[2, g, t * 128:(t + 1) * 128, :] for t in range(NT128)], axis=1)
            kv = jnp.dot(pkt, nat[1, g], preferred_element_type=F32)
            kvs.append(jnp.where(bd, kv, 0.0).astype(BF))
            z = jnp.sum(zacc[0, g], axis=0, keepdims=True)
            z16 = jnp.where(zr == zc, z, 0.0).astype(BF)
            for r in range(NQ):
                pq = jnp.concatenate(
                    [tt[3, g, (r * TPQ + t) * 128:(r * TPQ + t + 1) * 128, :] for t in range(TPQ)], axis=1)
                den = jnp.dot(z16, pq, preferred_element_type=F32)
                inv = 1.0 / (den[0:8, :] + 1e-6)
                pqf = pq.astype(F32)
                o_t = jnp.concatenate(
                    [pqf[j * DH:(j + 1) * DH, :] * inv[j:j + 1, :] for j in range(4)], axis=0)
                x[2, g, r * TQ:(r + 1) * TQ, :] = o_t.T.astype(BF)
            if g > 0:
                m_rows(g - 1)
        m_rows(G - 1)

    def out_slice(iu):
        g, qi = _divmod_pow2(iu, NQ)
        o_t = jnp.concatenate(
            [oacc[j] * (1.0 / jnp.sum(lbuf[j], axis=0, keepdims=True)) for j in range(4)], axis=0)
        wo = jnp.concatenate([w[7, c, _ds(g, 128), :] for c in range(G)], axis=1)
        y = lax.dot_general(o_t.astype(BF), wo, TN, preferred_element_type=F32)
        if isinstance(iu, int):
            obufa[qi] = (y + acca[qi]).astype(BF)
        else:
            acca[qi] = y + jnp.where(g == 0, 0.0, acca[qi])

    def stage(i1, i2, j, hook):
        sb = sbuf.at[j]
        if i1 is not None:
            g, qi = _divmod_pow2(i1, NQ)
            p1 = g & 1
            qh = jnp.concatenate(
                [cur[1, p1, _ds((qi * TPQ + t) * 4 + j, DH), :] for t in range(TPQ)], axis=1)
            zero = jnp.zeros((DH, TQ), BF)
            wq = jnp.concatenate([qh if jj == j else zero for jj in range(4)], axis=0)
        if i2 is not None:
            p2 = _divmod_pow2(i2, NQ)[0] & 1
            m_prev = jnp.max(mbuf[j], axis=0, keepdims=True)
        m8 = l8 = acc = None
        for c in range(NK):
            rows = slice(c * TK, (c + 1) * TK)
            if i1 is not None:
                st = jnp.dot(cur[0, p1, rows, :], wq, preferred_element_type=F32)
            if i2 is not None:
                p = jnp.exp2(sb[rows, :] - m_prev)
                ls = p.reshape(TK // 8, 8, TQ).sum(axis=0)
                l8 = ls if l8 is None else l8 + ls
                pb = p.astype(BF)
            if i1 is not None:
                sb[rows, :] = st
                mc = st.reshape(TK // 8, 8, TQ).max(axis=0)
                m8 = mc if m8 is None else jnp.maximum(m8, mc)
            hook(j, c)
            if i2 is not None:
                vh = jnp.concatenate(
                    [cur[2, p2, _ds((c * (TK // 128) + t) * 4 + j, DH), :] for t in range(TK // 128)], axis=1)
                o = jnp.dot(vh, pb, preferred_element_type=F32)
                acc = o if acc is None else o + acc
        if i2 is not None:
            lbuf[j] = l8
            oacc[j] = acc
        if i1 is not None:
            mbuf[j] = m8

    def make_hook(units, iu, slots):
        def hook(j, c):
            if (j, c) == OSLOT and iu is not None:
                out_slice(iu)
            for k, pos in enumerate(slots):
                if pos == (j, c) and k < len(units):
                    units[k]()
        return hook

    wait(cw1)
    with _scope('body0'):
        hook = make_hook([lambda u=u: unit(u) for u in SCHED[0]], None, SLOTS)
        for j in range(4):
            stage(0, None, j, hook)
    wait(cw2)

    def body(i, c):
        hook = make_hook([lambda k=k: unit(tab[i * NU + k]) for k in range(NU)], jnp.maximum(i - 2, 0), SLOTS)
        with _scope('bd'):
            for j in range(4):
                stage(i, i - 1, j, hook)

        g, qi = _divmod_pow2(i, NQ)

        @pl.when(g < G - 1)
        def _():
            @pl.when(qi == 1)
            def _():
                f_out(0, g + 1).start()
                f_out(1, g + 1).start()

            @pl.when(qi == 2)
            def _():
                f_out(2, g + 1).start()
                for k in range(2):
                    f_out(k, g + 1).wait()
                    f_in(k, g + 1).start()

            @pl.when(qi == 3)
            def _():
                f_out(2, g + 1).wait()
                f_in(2, g + 1).start()
                f_in(0, g + 1).wait()
                f_in(1, g + 1).wait()

        @pl.when(qi == 0)
        def _():
            f_in(2, g).wait()

        @pl.when(jnp.logical_or(i <= 3, i >= MID))
        def _():
            @pl.when(i == 1)
            def _():
                wait(cxb)
                wait(cw3)

            @pl.when(i == 3)
            def _():
                wait(cw4)

            @pl.when(i == MID)
            def _():
                with _scope('bmid'):
                    b_mid()

            @pl.when(i > MID)
            def _():
                def go(n, cc):
                    out_copy_b(n).start()
                    return cc
                lax.fori_loop(NU * (i - MID - 1), NU * (i - MID), go, 0)
        return c
    with _scope('attn'):
        lax.fori_loop(1, NB, body, 0)

    with _scope('epi'):
        n0 = NHB * G - NU_EPI
        n1 = EPI_FINE
        n2 = n1 + EPI_PRE
        for qi in range(NQ - 2):
            obufa[qi] = acca[qi].astype(BF)
        for qi in range(NQ - 2):
            out_copy_a(qi).start()
        part = {}

        def piece(n):
            k, rh, kh = n // 4, (n // 2) % 2, n % 2
            u = SCHED[NB][k]
            y = unit_mm(u, rh, kh)
            if kh == 0:
                part[0] = y
            else:
                nat[2, u[2], pl.ds(u[1] * HB + rh * 128, 128), :] = (y + part[0]).astype(BF)

        first = 4 * NK - 4 * n1

        def hook(j, c):
            if (j, c) == OSLOT:
                out_slice(NB - 2)
            if j * NK + c >= first:
                piece(j * NK + c - first)
        for j in range(4):
            stage(None, NB - 1, j, hook)
        out_copy_a(NQ - 2).start()
        for k in range(n1, n2):
            unit(SCHED[NB][k])
        out_slice(NB - 1)
        out_copy_a(NQ - 1).start()
        for k in range(n2):
            out_copy_b(n0 + k).start()
        for k in range(n2, NU_EPI):
            unit(SCHED[NB][k])
            out_copy_b(n0 + k).start()

    for r in range(NQ):
        out_copy_a(r).wait()
    for n in range(NHB * G):
        out_copy_b(n).wait()


@jax.jit
def pallas_concat_heads__mha_block__linear_attn_block__prompt_kernel(A_x, A_wqkv, A_wo, B_x, B_wqkv, B_wo):
    any_spec = pl.BlockSpec(memory_space=pl.ANY)
    return pl.pallas_call(
        _kernel,
        out_shape=jax.ShapeDtypeStruct((1, S, 2 * D), BF),
        in_specs=[any_spec] * 6,
        out_specs=any_spec,
        scratch_shapes=[
            pltpu.VMEM((3, G, S, 128), BF),
            pltpu.VMEM((8, G, D, 128), BF),
            pltpu.VMEM((4, G, S, 128), BF),
            pltpu.VMEM((5, G, S, 128), BF),
            pltpu.VMEM((3, 2, S, 128), BF),
            pltpu.VMEM((2, G, 8, 128), F32),
            pltpu.VMEM((4, S, TQ), F32),
            pltpu.VMEM((4, 8, TQ), F32),
            pltpu.VMEM((4, 8, TQ), F32),
            pltpu.VMEM((4, DH, TQ), F32),
            pltpu.VMEM((NQ, TQ, D), F32),
            pltpu.VMEM((NQ, TQ, D), BF),
            pltpu.SMEM((NB * NU,), jnp.int32),
            pltpu.SemaphoreType.DMA((10,)),
            pltpu.SemaphoreType.DMA((NQ + 1,)),
            pltpu.SemaphoreType.DMA((6,)),
        ],
        compiler_params=pltpu.CompilerParams(vmem_limit_bytes=120 * 1024 * 1024, disable_bounds_checks=True),
    )(A_x, A_wqkv, A_wo, B_x, B_wqkv, B_wo)
```

```python
import math
import jax
import jax.numpy as jnp
import numpy as np
from jax import lax
import jax.experimental.pallas as pl
import jax.experimental.pallas.tpu as pltpu

S, D, H, DH = 2048, 1024, 32, 32
G = D // 128
TQ = 512
TK = 128
NQ = S // TQ
NK = S // TK
TPQ = TQ // 128
NB = NQ * G
HB = 256
NHB = S // HB
NU = 14
NU_0 = 24
NU_EPI = 30
MID = 24
QSCALE = (DH ** -0.5) * math.log2(math.e)
BF = jnp.bfloat16
F32 = jnp.float32
SCOPES = False

X_A, X_B, O_B, O_A = 8, 9, 10, 11
U_SRC = (X_A, X_A, X_A, X_B, 3, X_B, O_B, O_A)
U_TR = (0, 1, 1, 1, 0, 1, 0, 0)
U_ACT = (0, 1, 0, 2, 0, 2, 0, 0)
SLOTS = [(j, c) for j in range(4) for c in (3, 7, 11, 15)][:NU]
SLOTS_0 = [(j, c) for j in range(4) for c in range(2, NK, 2)][:NU_0]
PR = 64
EPI_FINE = 8
NF = 7
NBF = 4
P1 = 3
ORDER = [(g, q) for g in range(G) for q in range(P1)] + [(g, NQ - 1) for g in range(G)]
RA = P1 * TQ // HB


def _schedule():
    a_units = [(k, r, g) for g in range(1, G) for k in (0, 1, 2) for r in range(NHB)]
    b_pre = [(k, r, c) for k in (3, 5, 4) for r in range(NHB) for c in range(G)]

    def late(c):
        return [(6, r, c) for r in range(NHB)] + [(7, r, c) for r in range(RA)]

    sched = [[a_units.pop(0) for _ in range(NU_0)]]
    for i in range(1, MID + 1):
        na = min(len(a_units), 8)
        sched.append([a_units.pop(0) for _ in range(na)] + [b_pre.pop(0) for _ in range(NU - na)])
    assert not a_units and not b_pre
    assert all(k < 3 and c == 1 for k, r, c in sched[0])
    for i in range(MID + 1, NB):
        sched.append(late(i - MID - 1))
    sched.append(late(G - 1) + [(7, r, c) for r in range(RA, NHB) for c in range(G)])
    assert all(len(us) == NU for us in sched[1:NB]) and len(sched[NB]) == NU_EPI
    done = set()
    for i in range(NB):
        for k, r, c in sched[i]:
            if k == 4:
                assert all((3, rr, cc) in done for rr in range(NHB) for cc in range(G))
            if k == 7:
                assert all(ORDER.index((g, r // 2)) + 2 <= i for g in range(G)), (i, r)
        assert i > 3 or all(c <= 2 if k < 3 else k == 3 for k, r, c in sched[i])
        done.update(sched[i])
        g = i // P1 + 1
        if g < G and i % P1 == 0:
            assert all((k, r, g) in done for k in (0, 1, 2) for r in range(NHB)), i
    return sched


SCHED = _schedule()


def _arow(slot, tile, row=0):
    return (slot * G + tile) * S + row


def _wrow(slot, tile, row=0):
    return (slot * G + tile) * D + row


def _fields(u):
    k, r, c = u
    wslot = 8 + r // (NHB // 2) if k == 4 else k
    if k == 3:
        dst = [_arow(3, t % G, (t // G) * D + c * 128) for t in (2 * r, 2 * r + 1)]
    else:
        dst = [_arow(k, c, r * HB), _arow(k, c, r * HB + 128)]
    return (_arow(U_SRC[k], 0, r * HB), _wrow(wslot, c), dst[0], dst[1],
            ((0 if k == 3 else G) + c) * 8, U_TR[k], U_ACT[k])


def _body_fields(i):
    g, q = ORDER[min(i, NB - 1)]
    g1 = ORDER[min(max(i - 1, 0), NB - 1)][0]
    g2, q2 = ORDER[max(i - 2, 0)]
    return _arow(0, g), _arow(1, g, q * TQ), _arow(2, g1), _arow(O_A, g2, q2 * TQ)


TB0 = NB * NU * NF
TAB_LEN = -(-(TB0 + NB * NBF) // 1024) * 1024


def _table():
    t = np.zeros((TAB_LEN,), np.int32)
    for i in range(1, NB):
        for k, u in enumerate(SCHED[i]):
            t[(i * NU + k) * NF:(i * NU + k + 1) * NF] = _fields(u)
        t[TB0 + i * NBF:TB0 + (i + 1) * NBF] = _body_fields(i)
    return t


class _Null:
    def __enter__(self):
        return self

    def __exit__(self, *a):
        return False


def _scope(name):
    return jax.named_scope(name) if SCOPES else _Null()


def _phi(t):
    return jnp.where(t > 0, t + 1.0, jnp.exp(t)) + 1e-6


def _rows(start, size, align=None):
    if isinstance(start, int):
        return pl.ds(start, size)
    return pl.ds(pl.multiple_of(start, align or size), size)


def _kernel(xa_h, wa_h, woa_h, xb_h, wb_h, wob_h, tab_h, out_h,
            a, w, cur, zacc, sbuf, mbuf, lbuf, oacc, tab, sem_in, sem_out, sem_f):
    def w_src(slot, c):
        cols = pl.ds(c * 128, 128)
        if slot < 3:
            return wa_h.at[:, pl.ds((1, 0, 2)[slot] * D + c * 128, 128)]
        if slot < 6:
            return wb_h.at[:, pl.ds((1, 2, 0)[slot - 3] * D + c * 128, 128)]
        if slot < 8:
            return (wob_h, woa_h)[slot - 6].at[:, cols]
        return xb_h.at[0, pl.ds((slot - 8) * D, D), cols]

    def cw(pairs, s):
        return [pltpu.make_async_copy(w_src(sl, c), w.at[pl.ds(_wrow(sl, c), D)], sem_in.at[s]) for sl, c in pairs]

    def cx(src, slot, row, n, s):
        return [pltpu.make_async_copy(src.at[0, pl.ds(row, n), pl.ds(k * 128, 128)],
                                      a.at[pl.ds(_arow(slot, k, row), n)], sem_in.at[s]) for k in range(G)]

    d1 = cw([(1, 0)], 0) + cx(xa_h, X_A, 0, HB, 0)
    d2 = cw([(2, 0), (0, 0)], 5)
    d3 = cx(xa_h, X_A, HB, HB, 11)
    dx = [None] + [cx(xa_h, X_A, r * TQ, TQ, r) for r in range(1, NQ)]
    cxb = cx(xb_h, X_B, 0, S, 4)
    cw1 = cw([(sl, c) for c in (1, 2) for sl in (0, 1, 2)], 6)
    cw2 = cw([(3, c) for c in range(G)], 7)
    cw3 = cw([(sl, c) for c in range(3, G) for sl in (0, 1, 2)], 8)
    cw4 = cw([(sl, c) for sl in (5, 8, 9, 4, 6, 7) for c in range(G)], 9)
    ctab = pltpu.make_async_copy(tab_h, tab, sem_in.at[10])

    def start(cs):
        for c in cs:
            c.start()

    def wait(cs):
        for c in cs:
            c.wait()

    def out_copy(k, c, row, n):
        return pltpu.make_async_copy(
            a.at[_rows(_arow(k, c, row), n, HB)],
            out_h.at[0, pl.ds(row, n), _rows((D if k == 6 else 0) + c * 128, 128)], sem_out.at[0])

    def late_copies(c):
        return [out_copy(6, c, 0, S), out_copy(7, c, 0, RA * HB)]

    def f_out(g):
        return [pltpu.make_async_copy(
            a.at[_rows(_arow(k, g), S)], out_h.at[0, :, pl.ds(k * 128, 128)], sem_f.at[0]) for k in range(3)]

    def f_in(g):
        return [pltpu.make_async_copy(
            out_h.at[0, :, pl.ds(k * 128, 128)], cur.at[_rows(_arow(k, g), S)], sem_f.at[1]) for k in range(3)]

    def unit_mm(u, rp, kh):
        xo, wo = _fields(u)[:2]
        ks = range(kh * G // 2, (kh + 1) * G // 2)
        lhs = jnp.concatenate([a[pl.ds(xo + k * S + rp * PR, PR), :] for k in ks], axis=1)
        return jnp.dot(lhs, w[pl.ds(wo + ks[0] * 128, D // 2), :], preferred_element_type=F32)

    def unit(fields, direct=False):
        xo, wo, r0, r1, zo, tr, act = fields
        static = isinstance(act, int)
        lhs = jnp.concatenate([a[_rows(xo + k * S, HB), :] for k in range(G)], axis=1)
        y = jnp.dot(lhs, w[_rows(wo, D), :], preferred_element_type=F32)
        if static:
            if act == 1:
                y = y * QSCALE
            elif act == 2:
                y = _phi(y)
        else:
            y = jnp.where(act == 2, _phi(y), y * jnp.where(act == 1, QSCALE, 1.0))
        if not static or zo < G * 8:
            zacc[_rows(zo, 8), :] += y.reshape(HB // 8, 8, 128).sum(axis=0)
        y_t = jnp.concatenate([y[t * 128:(t + 1) * 128, :].T for t in range(HB // 128)], axis=0)
        if static:
            out = (y_t if tr else y).astype(BF)
        else:
            out = jnp.where(tr == 1, y_t, y).astype(BF)
        dst = cur if direct else a
        dst[_rows(r0, 128), :] = out[:128]
        dst[_rows(r1, 128), :] = out[128:]

    def up_unit(k, r):
        unit(_fields((k, r, 0)), direct=True)

    start(d1)
    start(d2)
    start(d3)
    start(dx[1])
    zacc[...] = jnp.zeros_like(zacc)
    oacc[...] = jnp.zeros_like(oacc)
    lbuf[...] = jnp.ones_like(lbuf)

    def up_body(r, c):
        @pl.when(r == 1)
        def _():
            wait(dx[1])
            start(cw1)

        @pl.when(r == 2)
        def _():
            wait(dx[2])

        @pl.when(r == 3)
        def _():
            wait(dx[3])

        for k in (1, 2, 0):
            for hh in range(TQ // HB):
                up_unit(k, r * (TQ // HB) + hh)
        return c
    with _scope('upfront'):
        wait(d1)
        start(dx[2])
        up_unit(1, 0)
        wait(d2)
        start(dx[3])
        up_unit(2, 0)
        up_unit(0, 0)
        wait(d3)
        for k in (1, 2, 0):
            up_unit(k, 1)
        lax.fori_loop(1, NQ, up_body, 0)

    def b_mid():
        rr = lax.broadcasted_iota(jnp.int32, (128, 128), 0) // DH
        cc = lax.broadcasted_iota(jnp.int32, (128, 128), 1) // DH
        bd = rr == cc
        zr = lax.broadcasted_iota(jnp.int32, (16, 128), 0)
        zc = lax.broadcasted_iota(jnp.int32, (16, 128), 1) // DH
        kvs = {}

        def kv_half(g, h):
            cs = range(h * G // 2, (h + 1) * G // 2)
            kx = jnp.concatenate(
                [a[pl.ds(_arow(4, c, g * 128), 128), :].astype(F32)
                 + a[pl.ds(_arow(4, c, D + g * 128), 128), :].astype(F32) for c in cs], axis=1)
            return jnp.dot(kx.astype(BF), w[pl.ds(_wrow(4, g, cs[0] * 128), D // 2), :],
                           preferred_element_type=F32)

        def m_half(g, h):
            cs = range(h * G // 2, (h + 1) * G // 2)
            wo = jnp.concatenate([w[pl.ds(_wrow(6, c, g * 128), 128), :] for c in cs], axis=1)
            m = jnp.dot(kvs[g], wo, preferred_element_type=F32).astype(BF)
            for n, c in enumerate(cs):
                w[pl.ds(_wrow(6, c, g * 128), 128), :] = m[:, n * 128:(n + 1) * 128]

        def norm(g, r, z16):
            pq = jnp.concatenate(
                [a[pl.ds(_arow(5, g, (r * TPQ + t) * 128), 128), :] for t in range(TPQ)], axis=1)
            den = jnp.dot(z16, pq, preferred_element_type=F32)
            inv = 1.0 / (den[0:8, :] + 1e-6)
            pqf = pq.astype(F32)
            o_t = jnp.concatenate(
                [pqf[j * DH:(j + 1) * DH, :] * inv[j:j + 1, :] for j in range(4)], axis=0)
            a[pl.ds(_arow(O_B, g, r * TQ), TQ), :] = o_t.T.astype(BF)

        for g in range(G + 1):
            if g < G:
                z = jnp.sum(zacc[g * 8:(g + 1) * 8, :], axis=0, keepdims=True)
                z16 = jnp.where(zr == zc, z, 0.0).astype(BF)
                kv = kv_half(g, 0)
                norm(g, 0, z16)
                kv = kv_half(g, 1) + kv
                kvs[g] = jnp.where(bd, kv, 0.0).astype(BF)
                norm(g, 1, z16)
            for h in range(2):
                if g > 0:
                    m_half(g - 1, h)
                if g < G:
                    norm(g, 2 + h, z16)

    def o_store(o0):
        o_t = jnp.concatenate(
            [oacc[j] * (1.0 / jnp.sum(lbuf[j], axis=0, keepdims=True)) for j in range(4)], axis=0)
        a[_rows(o0, TQ), :] = o_t.T.astype(BF)

    def stage(k0, q0, v0, j, hook):
        sb = sbuf.at[j]
        if k0 is not None:
            qh = jnp.concatenate([cur[_rows(q0 + j * DH + t * 128, DH), :] for t in range(TPQ)], axis=1)
            zero = jnp.zeros((DH, TQ), BF)
            wq = jnp.concatenate([qh if jj == j else zero for jj in range(4)], axis=0)
        if v0 is not None:
            m_prev = jnp.max(mbuf[j], axis=0, keepdims=True)
        m8 = l8 = acc = None
        for c in range(NK):
            rows = slice(c * TK, (c + 1) * TK)
            hook(j, c)

            def qk():
                return jnp.dot(cur[_rows(k0 + c * TK, TK), :], wq, preferred_element_type=F32)
            early = k0 is not None and (j, c) < SLOTS[0]
            if early:
                st = qk()
            if v0 is not None:
                p = jnp.exp2(sb[rows, :] - m_prev)
                for r in reversed(range(TK // 16)):
                    pr = p[r * 16:r * 16 + 8, :] + p[r * 16 + 8:r * 16 + 16, :]
                    l8 = pr if l8 is None else l8 + pr
                o = jnp.dot(cur[_rows(v0 + j * DH + c * TK, DH), :], p.astype(BF), preferred_element_type=F32)
                acc = o if acc is None else o + acc
            if k0 is not None:
                if not early:
                    st = qk()
                sb[rows, :] = st
                mc = st.reshape(TK // 8, 8, TQ).max(axis=0)
                m8 = mc if m8 is None else jnp.maximum(m8, mc)
        if v0 is not None:
            lbuf[j] = l8
            oacc[j] = acc
        if k0 is not None:
            mbuf[j] = m8

    def make_hook(units, slots, o0=None, extra=None):
        def hook(j, c):
            if (j, c) == (0, 2) and extra is not None:
                extra()
            for k, pos in enumerate(slots):
                if pos == (j, c):
                    units[k]()
            if (j, c) == (0, 0) and o0 is not None:
                o_store(o0)
        return hook

    wait(cw1)
    with _scope('body0'):
        hook = make_hook([lambda u=u: unit(_fields(u), direct=True) for u in SCHED[0]], SLOTS_0)
        k0, q0 = _body_fields(0)[:2]
        for j in range(4):
            stage(k0, q0, None, j, hook)
            if j == 0:
                ctab.start()
                start(cxb)
                start(cw2)
            if j == 2:
                start(cw3)
                start(cw4)
    wait(cxb)
    wait(cw2)
    ctab.wait()

    def body(i, carry):
        ph, g, act = carry
        t0 = i * (NU * NF)
        k0, q0, v0, o0 = (tab[TB0 + i * NBF + n] for n in range(4))
        hook = make_hook([lambda k=k: unit(tuple(tab[t0 + k * NF + n] for n in range(NF))) for k in range(NU)],
                         SLOTS, o0, lambda: pl.when(act == 2)(lambda: start(f_in(g + 1))))

        @pl.when(act == 1)
        def _():
            wait(f_in(g))

        @pl.when(act == 2)
        def _():
            wait(f_out(g + 1))

        with _scope('bd'):
            for j in range(4):
                stage(k0, q0, v0, j, hook)

        @pl.when(jnp.logical_and(g < G - 1, ph == 0))
        def _():
            start(f_out(g + 1))

        @pl.when(i > MID)
        def _():
            start(late_copies(i - MID - 1))

        @pl.when(jnp.logical_or(i == 3, i == MID))
        def _():
            @pl.when(i == 3)
            def _():
                wait(cw3)
                wait(cw4)

            @pl.when(i == MID)
            def _():
                with _scope('bmid'):
                    b_mid()
        wrap = ph == P1 - 1
        act = jnp.where(jnp.logical_and(g >= 1, g < G - 1), jnp.where(wrap, 1, jnp.where(ph == 1, 2, 0)), 0)
        return jnp.where(wrap, 0, ph + 1), jnp.where(wrap, g + 1, g), act
    with _scope('attn'):
        lax.fori_loop(1, NB, body, (jnp.int32(1), jnp.int32(0), jnp.int32(0)))

    eu = SCHED[NB]

    def epi_copy(k):
        return out_copy(eu[k][0], eu[k][2], eu[k][1] * HB, HB)

    with _scope('epi'):
        part = {}
        npc = 2 * HB // PR

        def piece(n):
            k, rp, kh = n // npc, (n % npc) // 2, n % 2
            y = unit_mm(eu[k], rp, kh)
            if kh == 0:
                part[0] = y
            else:
                a[pl.ds(_fields(eu[k])[2] + rp * PR, PR), :] = (y + part[0]).astype(BF)
            if n % npc == npc - 1:
                epi_copy(k).start()

        def hook(j, c):
            n = j * NK + c
            for m in range(n * EPI_FINE * npc // (4 * NK), (n + 1) * EPI_FINE * npc // (4 * NK)):
                piece(m)

        _, _, v0, o0 = _body_fields(NB)
        o_store(o0)
        for j in range(4):
            stage(None, None, v0, j, hook)
        o_store(_body_fields(NB + 1)[3])
        for k in range(EPI_FINE, NU_EPI):
            unit(_fields(eu[k]))
            epi_copy(k).start()

    for c in range(G - 1):
        wait(late_copies(c))
    for k in range(NU_EPI):
        epi_copy(k).wait()


@jax.jit
def pallas_concat_heads__mha_block__linear_attn_block__prompt_kernel(A_x, A_wqkv, A_wo, B_x, B_wqkv, B_wo):
    any_spec = pl.BlockSpec(memory_space=pl.ANY)
    return pl.pallas_call(
        _kernel,
        out_shape=jax.ShapeDtypeStruct((1, S, 2 * D), BF),
        in_specs=[any_spec] * 7,
        out_specs=any_spec,
        scratch_shapes=[
            pltpu.VMEM((12 * G * S, 128), BF),
            pltpu.VMEM((10 * G * D, 128), BF),
            pltpu.VMEM((3 * G * S, 128), BF),
            pltpu.VMEM((2 * G * 8, 128), F32),
            pltpu.VMEM((4, S, TQ), F32),
            pltpu.VMEM((4, 8, TQ), F32),
            pltpu.VMEM((4, 8, TQ), F32),
            pltpu.VMEM((4, DH, TQ), F32),
            pltpu.SMEM((TAB_LEN,), jnp.int32),
            pltpu.SemaphoreType.DMA((12,)),
            pltpu.SemaphoreType.DMA((1,)),
            pltpu.SemaphoreType.DMA((2,)),
        ],
        compiler_params=pltpu.CompilerParams(vmem_limit_bytes=120 * 1024 * 1024, disable_bounds_checks=True),
    )(A_x, A_wqkv, A_wo, B_x, B_wqkv, B_wo, jnp.asarray(_table()))
```

```python
import math
import jax
import jax.numpy as jnp
import numpy as np
from jax import lax
import jax.experimental.pallas as pl
import jax.experimental.pallas.tpu as pltpu

S, D, H, DH = 2048, 1024, 32, 32
G = D // 128
TQ = 512
TK = 128
NQ = S // TQ
NK = S // TK
TPQ = TQ // 128
NB = NQ * G
HB = 256
NHB = S // HB
NU = 14
NU_0 = 24
NU_EPI = 30
MID = 24
QSCALE = (DH ** -0.5) * math.log2(math.e)
BF = jnp.bfloat16
F32 = jnp.float32

X_A, X_B, O_B, O_A = 8, 9, 10, 11
U_SRC = (X_A, X_A, X_A, X_B, 3, X_B, O_B, O_A)
U_TR = (0, 1, 1, 1, 0, 1, 0, 0)
U_ACT = (0, 1, 0, 2, 0, 2, 0, 0)
SLOTS = [(j, c) for j in range(4) for c in (3, 7, 11, 15)][:NU]
SLOTS_0 = ([(0, c) for c in (1, 2, 3, 4)] + [(j, c) for j in range(4) for c in range(2, NK, 2)][2:])[:NU_0]
PR = 64
EPI_FINE = 8
NF = 7
NBF = 4
P1 = 3
ORDER = [(g, q) for g in range(G) for q in range(P1)] + [(g, NQ - 1) for g in range(G)]
RA = P1 * TQ // HB


def _schedule():
    a_units = ([(k, r, g) for g in (0, 1) for k in (0, 2, 1) for r in range(NHB // 2, NHB)]
               + [(k, r, g) for g in range(2, G) for k in (0, 1, 2) for r in range(NHB)])
    b_pre = [(k, r, c) for k in (3, 5, 4) for r in range(NHB) for c in range(G)]

    def late(c):
        return [(6, r, c) for r in range(NHB)] + [(7, r, c) for r in range(RA)]

    sched = [[a_units.pop(0) for _ in range(NU_0)]]
    for i in range(1, MID + 1):
        na = min(len(a_units), 8)
        sched.append([a_units.pop(0) for _ in range(na)] + [b_pre.pop(0) for _ in range(NU - na)])
    assert not a_units and not b_pre
    assert all(k < 3 and c <= 1 for k, r, c in sched[0])
    for i in range(MID + 1, NB):
        sched.append(late(i - MID - 1))
    sched.append(late(G - 1) + [(7, r, c) for r in range(RA, NHB) for c in range(G)])
    assert all(len(us) == NU for us in sched[1:NB]) and len(sched[NB]) == NU_EPI
    done = set((k, r, g) for k in range(3) for r in range(NHB // 2) for g in (0, 1))
    for i in range(NB):
        for k, r, c in sched[i]:
            if k == 4:
                assert all((3, rr, cc) in done for rr in range(NHB) for cc in range(G))
            if k == 7:
                assert all(ORDER.index((g, r // 2)) + 2 <= i for g in range(G)), (i, r)
        assert i > 3 or all(c <= 2 if k < 3 else k == 3 for k, r, c in sched[i])
        done.update(sched[i])
        g = i // P1 + 1
        if g < G and i % P1 == 0:
            assert all((k, r, g) in done for k in (0, 1, 2) for r in range(NHB)), i
    return sched


SCHED = _schedule()


def _arow(slot, tile, row=0):
    return (slot * G + tile) * S + row


def _wrow(slot, tile, row=0):
    return (slot * G + tile) * D + row


def _fields(u):
    k, r, c = u
    wslot = 8 + r // (NHB // 2) if k == 4 else k
    if k == 3:
        dst = [_arow(3, t % G, (t // G) * D + c * 128) for t in (2 * r, 2 * r + 1)]
    else:
        dst = [_arow(k, c, r * HB), _arow(k, c, r * HB + 128)]
    return (_arow(U_SRC[k], 0, r * HB), _wrow(wslot, c), dst[0], dst[1],
            ((0 if k == 3 else G) + c) * 8, U_TR[k], U_ACT[k])


def _body_fields(i):
    g, q = ORDER[min(i, NB - 1)]
    g1 = ORDER[min(max(i - 1, 0), NB - 1)][0]
    g2, q2 = ORDER[max(i - 2, 0)]
    return _arow(0, g), _arow(1, g, q * TQ), _arow(2, g1), _arow(O_A, g2, q2 * TQ)


TB0 = NB * NU * NF
TAB_LEN = -(-(TB0 + NB * NBF) // 1024) * 1024


def _table():
    t = np.zeros((TAB_LEN,), np.int32)
    for i in range(1, NB):
        for k, u in enumerate(SCHED[i]):
            t[(i * NU + k) * NF:(i * NU + k + 1) * NF] = _fields(u)
        t[TB0 + i * NBF:TB0 + (i + 1) * NBF] = _body_fields(i)
    return t


def _phi(t):
    return jnp.where(t > 0, t + 1.0, jnp.exp(t)) + 1e-6


def _rows(start, size, align=None):
    if isinstance(start, int):
        return pl.ds(start, size)
    return pl.ds(pl.multiple_of(start, align or size), size)


def _kernel(xa_h, wa_h, woa_h, xb_h, wb_h, wob_h, tab_h, out_h,
            a, w, cur, zacc, sbuf, mbuf, lbuf, oacc, tab, sem_in, sem_out, sem_f):
    def w_src(slot, c):
        cols = pl.ds(c * 128, 128)
        if slot < 3:
            return wa_h.at[:, pl.ds((1, 0, 2)[slot] * D + c * 128, 128)]
        if slot < 6:
            return wb_h.at[:, pl.ds((1, 2, 0)[slot - 3] * D + c * 128, 128)]
        if slot < 8:
            return (wob_h, woa_h)[slot - 6].at[:, cols]
        return xb_h.at[0, pl.ds((slot - 8) * D, D), cols]

    def cw(pairs, s):
        return [pltpu.make_async_copy(w_src(sl, c), w.at[pl.ds(_wrow(sl, c), D)], sem_in.at[s]) for sl, c in pairs]

    def cx(src, slot, row, n, s):
        return [pltpu.make_async_copy(src.at[0, pl.ds(row, n), pl.ds(k * 128, 128)],
                                      a.at[pl.ds(_arow(slot, k, row), n)], sem_in.at[s]) for k in range(G)]

    d1 = cw([(1, 0)], 0) + cx(xa_h, X_A, 0, HB, 0)
    d2 = cw([(2, 0), (0, 0)], 5)
    d3 = cx(xa_h, X_A, HB, HB, 11)
    dx = [None] + [cx(xa_h, X_A, r * TQ, TQ, r) for r in range(1, NQ)]
    cxb = cx(xb_h, X_B, 0, S, 4)
    cw1 = cw([(sl, 1) for sl in (0, 1, 2)], 6)
    cw2 = cw([(sl, 2) for sl in (0, 1, 2)] + [(3, c) for c in range(G)], 7)
    cw3 = cw([(sl, c) for c in range(3, G) for sl in (0, 1, 2)], 8)
    cw4 = cw([(sl, c) for sl in (5, 8, 9, 4, 6, 7) for c in range(G)], 9)
    ctab = pltpu.make_async_copy(tab_h, tab, sem_in.at[10])

    def start(cs):
        for c in cs:
            c.start()

    def wait(cs):
        for c in cs:
            c.wait()

    def out_copy(k, c, row, n):
        return pltpu.make_async_copy(
            a.at[_rows(_arow(k, c, row), n, HB)],
            out_h.at[0, pl.ds(row, n), _rows((D if k == 6 else 0) + c * 128, 128)], sem_out.at[0])

    def late_copies(c):
        return [out_copy(6, c, 0, S), out_copy(7, c, 0, RA * HB)]

    def f_out(g):
        return [pltpu.make_async_copy(
            a.at[_rows(_arow(k, g), S)], out_h.at[0, :, pl.ds(k * 128, 128)], sem_f.at[0]) for k in range(3)]

    def f_in(g):
        return [pltpu.make_async_copy(
            out_h.at[0, :, pl.ds(k * 128, 128)], cur.at[_rows(_arow(k, g), S)], sem_f.at[1]) for k in range(3)]

    def unit_mm(u, rp, kh):
        xo, wo = _fields(u)[:2]
        ks = range(kh * G // 2, (kh + 1) * G // 2)
        lhs = jnp.concatenate([a[pl.ds(xo + k * S + rp * PR, PR), :] for k in ks], axis=1)
        return jnp.dot(lhs, w[pl.ds(wo + ks[0] * 128, D // 2), :], preferred_element_type=F32)

    def unit(fields, direct=False):
        xo, wo, r0, r1, zo, tr, act = fields
        static = isinstance(act, int)
        lhs = jnp.concatenate([a[_rows(xo + k * S, HB), :] for k in range(G)], axis=1)
        y = jnp.dot(lhs, w[_rows(wo, D), :], preferred_element_type=F32)
        if static:
            if act == 1:
                y = y * QSCALE
            elif act == 2:
                y = _phi(y)
        else:
            y = jnp.where(act == 2, _phi(y), y * jnp.where(act == 1, QSCALE, 1.0))
        if not static or (isinstance(zo, int) and zo < G * 8):
            zacc[_rows(zo, 8), :] += y.reshape(HB // 8, 8, 128).sum(axis=0)
        y_t = jnp.concatenate([y[t * 128:(t + 1) * 128, :].T for t in range(HB // 128)], axis=0)
        if static:
            out = (y_t if tr else y).astype(BF)
        else:
            out = jnp.where(tr == 1, y_t, y).astype(BF)
        dst = cur if direct else a
        dst[_rows(r0, 128), :] = out[:128]
        dst[_rows(r1, 128), :] = out[128:]

    def up_unit(k, r, g=0):
        unit(_fields((k, r, g)), direct=True)

    ctab.start()
    start(d1)
    start(d2)
    start(d3)
    start(cw1)
    zacc[...] = jnp.zeros_like(zacc)
    oacc[...] = jnp.zeros_like(oacc)
    lbuf[...] = jnp.ones_like(lbuf)

    def up_body(n, c):
        @pl.when(n == 1)
        def _():
            wait(cw1)

        @pl.when(n == 2)
        def _():
            wait(dx[1])

        for k in (1, 2, 0):
            for hh in range(TQ // HB):
                up_unit(k, lax.shift_right_logical(n, 1) * (TQ // HB) + hh, n & 1)
        return c
    ctab.wait()
    wait(d1)
    start(dx[1])
    up_unit(1, 0)
    wait(d2)
    start(dx[2])
    up_unit(2, 0)
    up_unit(0, 0)
    wait(d3)
    start(dx[3])
    for k in (1, 2, 0):
        up_unit(k, 1)
    lax.fori_loop(1, 4, up_body, 0)

    def b_mid():
        rr = lax.broadcasted_iota(jnp.int32, (128, 128), 0) // DH
        cc = lax.broadcasted_iota(jnp.int32, (128, 128), 1) // DH
        bd = rr == cc
        zr = lax.broadcasted_iota(jnp.int32, (16, 128), 0)
        zc = lax.broadcasted_iota(jnp.int32, (16, 128), 1) // DH
        kvs = {}

        def kv_half(g, h):
            cs = range(h * G // 2, (h + 1) * G // 2)
            kx = jnp.concatenate(
                [a[pl.ds(_arow(4, c, g * 128), 128), :].astype(F32)
                 + a[pl.ds(_arow(4, c, D + g * 128), 128), :].astype(F32) for c in cs], axis=1)
            return jnp.dot(kx.astype(BF), w[pl.ds(_wrow(4, g, cs[0] * 128), D // 2), :],
                           preferred_element_type=F32)

        def m_half(g, h):
            cs = range(h * G // 2, (h + 1) * G // 2)
            wo = jnp.concatenate([w[pl.ds(_wrow(6, c, g * 128), 128), :] for c in cs], axis=1)
            m = jnp.dot(kvs[g], wo, preferred_element_type=F32).astype(BF)
            for n, c in enumerate(cs):
                w[pl.ds(_wrow(6, c, g * 128), 128), :] = m[:, n * 128:(n + 1) * 128]

        def norm(g, r, z16):
            pq = jnp.concatenate(
                [a[pl.ds(_arow(5, g, (r * TPQ + t) * 128), 128), :] for t in range(TPQ)], axis=1)
            den = jnp.dot(z16, pq, preferred_element_type=F32)
            inv = 1.0 / (den[0:8, :] + 1e-6)
            pqf = pq.astype(F32)
            o_t = jnp.concatenate(
                [pqf[j * DH:(j + 1) * DH, :] * inv[j:j + 1, :] for j in range(4)], axis=0)
            a[pl.ds(_arow(O_B, g, r * TQ), TQ), :] = o_t.T.astype(BF)

        for g in range(G + 1):
            if g < G:
                z = jnp.sum(zacc[g * 8:(g + 1) * 8, :], axis=0, keepdims=True)
                z16 = jnp.where(zr == zc, z, 0.0).astype(BF)
                kv = kv_half(g, 0)
                norm(g, 0, z16)
                kv = kv_half(g, 1) + kv
                kvs[g] = jnp.where(bd, kv, 0.0).astype(BF)
                norm(g, 1, z16)
            for h in range(2):
                if g > 0:
                    m_half(g - 1, h)
                if g < G:
                    norm(g, 2 + h, z16)

    def o_store(o0):
        o_t = jnp.concatenate(
            [oacc[j] * (1.0 / jnp.sum(lbuf[j], axis=0, keepdims=True)) for j in range(4)], axis=0)
        a[_rows(o0, TQ), :] = o_t.T.astype(BF)

    def stage(k0, q0, v0, j, hook):
        sb = sbuf.at[j]
        if k0 is not None:
            qh = jnp.concatenate([cur[_rows(q0 + j * DH + t * 128, DH), :] for t in range(TPQ)], axis=1)
            zero = jnp.zeros((DH, TQ), BF)
            wq = jnp.concatenate([qh if jj == j else zero for jj in range(4)], axis=0)
        if v0 is not None:
            m_prev = jnp.max(mbuf[j], axis=0, keepdims=True)
        m8 = l8 = acc = None
        for c in range(NK):
            rows = slice(c * TK, (c + 1) * TK)
            hook(j, c)

            def qk():
                return jnp.dot(cur[_rows(k0 + c * TK, TK), :], wq, preferred_element_type=F32)
            early = k0 is not None and (j, c) < SLOTS[0]
            if early:
                st = qk()
            if v0 is not None:
                p = jnp.exp2(sb[rows, :] - m_prev)
                for r in reversed(range(TK // 16)):
                    pr = p[r * 16:r * 16 + 8, :] + p[r * 16 + 8:r * 16 + 16, :]
                    l8 = pr if l8 is None else l8 + pr
                o = jnp.dot(cur[_rows(v0 + j * DH + c * TK, DH), :], p.astype(BF), preferred_element_type=F32)
                acc = o if acc is None else o + acc
            if k0 is not None:
                if not early:
                    st = qk()
                sb[rows, :] = st
                mc = st.reshape(TK // 8, 8, TQ).max(axis=0)
                m8 = mc if m8 is None else jnp.maximum(m8, mc)
        if v0 is not None:
            lbuf[j] = l8
            oacc[j] = acc
        if k0 is not None:
            mbuf[j] = m8

    def make_hook(units, slots, o0=None, extra=None):
        def hook(j, c):
            if (j, c) == (0, 2) and extra is not None:
                extra()
            for k, pos in enumerate(slots):
                if pos == (j, c):
                    units[k]()
            if (j, c) == (0, 0) and o0 is not None:
                o_store(o0)
        return hook

    wait(dx[2])
    wait(dx[3])
    start(cxb)
    start(cw2)
    hook = make_hook([lambda u=u: unit(_fields(u), direct=True) for u in SCHED[0]], SLOTS_0)
    k0, q0 = _body_fields(0)[:2]
    for j in range(4):
        stage(k0, q0, None, j, hook)
        if j == 2:
            start(cw3)
            start(cw4)
    wait(cxb)
    wait(cw2)

    def body(i, carry):
        ph, g, act = carry
        t0 = i * (NU * NF)
        k0, q0, v0, o0 = (tab[TB0 + i * NBF + n] for n in range(4))
        hook = make_hook([lambda k=k: unit(tuple(tab[t0 + k * NF + n] for n in range(NF))) for k in range(NU)],
                         SLOTS, o0, lambda: pl.when(act == 2)(lambda: start(f_in(g + 1))))

        @pl.when(act == 1)
        def _():
            wait(f_in(g))

        @pl.when(act == 2)
        def _():
            wait(f_out(g + 1))

        for j in range(4):
            stage(k0, q0, v0, j, hook)

        @pl.when(jnp.logical_and(g < G - 1, ph == 0))
        def _():
            start(f_out(g + 1))

        @pl.when(i > MID)
        def _():
            start(late_copies(i - MID - 1))

        @pl.when(jnp.logical_or(i == 3, i == MID))
        def _():
            @pl.when(i == 3)
            def _():
                wait(cw3)
                wait(cw4)

            @pl.when(i == MID)
            def _():
                b_mid()
        wrap = ph == P1 - 1
        act = jnp.where(jnp.logical_and(g >= 1, g < G - 1), jnp.where(wrap, 1, jnp.where(ph == 1, 2, 0)), 0)
        return jnp.where(wrap, 0, ph + 1), jnp.where(wrap, g + 1, g), act
    lax.fori_loop(1, NB, body, (jnp.int32(1), jnp.int32(0), jnp.int32(0)))

    eu = SCHED[NB]

    def epi_copy(k):
        return out_copy(eu[k][0], eu[k][2], eu[k][1] * HB, HB)

    part = {}
    npc = 2 * HB // PR

    def piece(n):
        k, rp, kh = n // npc, (n % npc) // 2, n % 2
        y = unit_mm(eu[k], rp, kh)
        if kh == 0:
            part[0] = y
        else:
            a[pl.ds(_fields(eu[k])[2] + rp * PR, PR), :] = (y + part[0]).astype(BF)
        if n % npc == npc - 1:
            epi_copy(k).start()

    def hook(j, c):
        n = j * NK + c
        for m in range(n * EPI_FINE * npc // (4 * NK), (n + 1) * EPI_FINE * npc // (4 * NK)):
            piece(m)

    _, _, v0, o0 = _body_fields(NB)
    o_store(o0)
    for j in range(4):
        stage(None, None, v0, j, hook)
    o_store(_body_fields(NB + 1)[3])
    for k in range(EPI_FINE, NU_EPI):
        unit(_fields(eu[k]))
        epi_copy(k).start()

    for c in range(G - 1):
        wait(late_copies(c))
    for k in range(NU_EPI):
        epi_copy(k).wait()


@jax.jit
def pallas_concat_heads__mha_block__linear_attn_block__prompt_kernel(A_x, A_wqkv, A_wo, B_x, B_wqkv, B_wo):
    any_spec = pl.BlockSpec(memory_space=pl.ANY)
    return pl.pallas_call(
        _kernel,
        out_shape=jax.ShapeDtypeStruct((1, S, 2 * D), BF),
        in_specs=[any_spec] * 7,
        out_specs=any_spec,
        scratch_shapes=[
            pltpu.VMEM((12 * G * S, 128), BF),
            pltpu.VMEM((10 * G * D, 128), BF),
            pltpu.VMEM((3 * G * S, 128), BF),
            pltpu.VMEM((2 * G * 8, 128), F32),
            pltpu.VMEM((4, S, TQ), F32),
            pltpu.VMEM((4, 8, TQ), F32),
            pltpu.VMEM((4, 8, TQ), F32),
            pltpu.VMEM((4, DH, TQ), F32),
            pltpu.SMEM((TAB_LEN,), jnp.int32),
            pltpu.SemaphoreType.DMA((12,)),
            pltpu.SemaphoreType.DMA((1,)),
            pltpu.SemaphoreType.DMA((2,)),
        ],
        compiler_params=pltpu.CompilerParams(vmem_limit_bytes=120 * 1024 * 1024, disable_bounds_checks=True,
                                             disable_semaphore_checks=True),
    )(A_x, A_wqkv, A_wo, B_x, B_wqkv, B_wo, jnp.asarray(_table()))
```

```python
import math
import jax
import jax.numpy as jnp
import numpy as np
from jax import lax
import jax.experimental.pallas as pl
import jax.experimental.pallas.tpu as pltpu

S, D, H, DH = 2048, 1024, 32, 32
G = D // 128
TQ = 512
TK = 128
NQ = S // TQ
NK = S // TK
TPQ = TQ // 128
NB = NQ * G
HB = 256
NHB = S // HB
NU = 14
NU_0 = 24
NU_EPI = 30
MID = 24
QSCALE = (DH ** -0.5) * math.log2(math.e)
BF = jnp.bfloat16
F32 = jnp.float32

X_A, X_B, O_B, O_A = 8, 9, 10, 11
U_SRC = (X_A, X_A, X_A, X_B, 3, X_B, O_B, O_A)
U_TR = (0, 1, 1, 1, 0, 1, 0, 0)
U_ACT = (0, 1, 0, 2, 0, 2, 0, 0)
SLOTS = [(j, c) for j in range(4) for c in (3, 7, 11, 15)][:NU]
SLOTS_0 = ([(0, c) for c in (1, 2, 3, 4)] + [(j, c) for j in range(4) for c in range(2, NK, 2)][2:])[:NU_0]
PR = 64
EPI_FINE = 8
NMID = 4
NF = 7
NBF = 4
P1 = 3
ORDER = [(g, q) for g in range(G) for q in range(P1)] + [(g, NQ - 1) for g in range(G)]
RA = P1 * TQ // HB


def _schedule():
    a_units = ([(k, r, g) for g in (0, 1) for k in (0, 2, 1) for r in range(NHB // 2, NHB)]
               + [(k, r, g) for g in range(2, G) for k in (0, 1, 2) for r in range(NHB)])
    b_pre = [(k, r, c) for k in (3, 5, 4) for r in range(NHB) for c in range(G)]

    def late(c):
        return [(6, r, c) for r in range(NHB)] + [(7, r, c) for r in range(RA)]

    sched = [[a_units.pop(0) for _ in range(NU_0)]]
    for i in range(1, MID + 1):
        na = min(len(a_units), 8)
        sched.append([a_units.pop(0) for _ in range(na)] + [b_pre.pop(0) for _ in range(NU - na)])
    assert not a_units and not b_pre
    assert all(k < 3 and c <= 1 for k, r, c in sched[0])
    for i in range(MID + 1, NB):
        sched.append(late(i - MID - 1))
    last = late(G - 1)
    last = last[NHB:NHB + NMID] + last[:NHB] + last[NHB + NMID:]
    sched.append(last + [(7, r, c) for r in range(RA, NHB) for c in range(G)])
    assert all(ORDER.index((g, r // 2)) + 2 <= MID for k, r, c in last[:NMID] for g in range(G))
    assert all(len(us) == NU for us in sched[1:NB]) and len(sched[NB]) == NU_EPI
    done = set((k, r, g) for k in range(3) for r in range(NHB // 2) for g in (0, 1))
    for i in range(NB):
        for k, r, c in sched[i]:
            if k == 4:
                assert all((3, rr, cc) in done for rr in range(NHB) for cc in range(G))
            if k == 7:
                assert all(ORDER.index((g, r // 2)) + 2 <= i for g in range(G)), (i, r)
        assert i > 3 or all(c <= 2 if k < 3 else k == 3 for k, r, c in sched[i])
        done.update(sched[i])
        g = i // P1 + 1
        if g < G and i % P1 == 0:
            assert all((k, r, g) in done for k in (0, 1, 2) for r in range(NHB)), i
    return sched


SCHED = _schedule()


def _arow(slot, tile, row=0):
    return (slot * G + tile) * S + row


def _wrow(slot, tile, row=0):
    return (slot * G + tile) * D + row


def _fields(u):
    k, r, c = u
    wslot = 8 + r // (NHB // 2) if k == 4 else k
    if k == 3:
        dst = [_arow(3, t % G, (t // G) * D + c * 128) for t in (2 * r, 2 * r + 1)]
    else:
        dst = [_arow(k, c, r * HB), _arow(k, c, r * HB + 128)]
    return (_arow(U_SRC[k], 0, r * HB), _wrow(wslot, c), dst[0], dst[1],
            ((0 if k == 3 else G) + c) * 8, U_TR[k], U_ACT[k])


def _body_fields(i):
    g, q = ORDER[min(i, NB - 1)]
    g1 = ORDER[min(max(i - 1, 0), NB - 1)][0]
    g2, q2 = ORDER[max(i - 2, 0)]
    return _arow(0, g), _arow(1, g, q * TQ), _arow(2, g1), _arow(O_A, g2, q2 * TQ)


TB0 = NB * NU * NF
TAB_LEN = -(-(TB0 + NB * NBF) // 1024) * 1024


def _table():
    t = np.zeros((TAB_LEN,), np.int32)
    for i in range(1, NB):
        for k, u in enumerate(SCHED[i]):
            t[(i * NU + k) * NF:(i * NU + k + 1) * NF] = _fields(u)
        t[TB0 + i * NBF:TB0 + (i + 1) * NBF] = _body_fields(i)
    return t


def _phi(t):
    return jnp.where(t > 0, t + 1.0, jnp.exp(t)) + 1e-6


def _rows(start, size, align=None):
    if isinstance(start, int):
        return pl.ds(start, size)
    return pl.ds(pl.multiple_of(start, align or size), size)


def _kernel(xa_h, wa_h, woa_h, xb_h, wb_h, wob_h, tab_h, out_h,
            a, w, cur, zacc, sbuf, mbuf, lbuf, oacc, tab, sem):
    def w_src(slot, c):
        cols = pl.ds(c * 128, 128)
        if slot < 3:
            return wa_h.at[:, pl.ds((1, 0, 2)[slot] * D + c * 128, 128)]
        if slot < 6:
            return wb_h.at[:, pl.ds((1, 2, 0)[slot - 3] * D + c * 128, 128)]
        if slot < 8:
            return (wob_h, woa_h)[slot - 6].at[:, cols]
        return xb_h.at[0, pl.ds((slot - 8) * D, D), cols]

    def cw(pairs, s):
        return [pltpu.make_async_copy(w_src(sl, c), w.at[pl.ds(_wrow(sl, c), D)], sem.at[s]) for sl, c in pairs]

    def cx(src, slot, row, n, s):
        return [pltpu.make_async_copy(src.at[0, pl.ds(row, n), pl.ds(k * 128, 128)],
                                      a.at[pl.ds(_arow(slot, k, row), n)], sem.at[s]) for k in range(G)]

    d1 = cw([(1, 0)], 0) + cx(xa_h, X_A, 0, HB, 0)
    d2 = cw([(2, 0), (0, 0)], 1)
    d3 = cx(xa_h, X_A, HB, HB, 2)
    cw1 = cw([(sl, 1) for sl in (0, 1, 2)], 3)
    ctab = pltpu.make_async_copy(tab_h, tab, sem.at[4])
    dx = [None] + [cx(xa_h, X_A, r * TQ, TQ, r - 1) for r in range(1, NQ)]
    cw2 = cx(xb_h, X_B, 0, S, 3) + cw([(sl, 2) for sl in (0, 1, 2)] + [(3, c) for c in range(G)], 3)
    cw3 = cw([(sl, c) for c in range(3, G) for sl in (0, 1, 2)]
             + [(sl, c) for sl in (5, 8, 9, 4, 6, 7) for c in range(G)], 4)

    def start(cs):
        for c in cs:
            c.start()

    def wait(cs):
        for c in cs:
            c.wait()

    def out_copy(k, c, row, n):
        return pltpu.make_async_copy(
            a.at[_rows(_arow(k, c, row), n, HB)],
            out_h.at[0, pl.ds(row, n), _rows((D if k == 6 else 0) + c * 128, 128)], sem.at[2])

    def late_copies(c):
        return [out_copy(6, c, 0, S), out_copy(7, c, 0, RA * HB)]

    def f_out(g):
        return [pltpu.make_async_copy(
            a.at[_rows(_arow(k, g), S)], out_h.at[0, :, pl.ds(k * 128, 128)], sem.at[0]) for k in range(3)]

    def f_in(g):
        return [pltpu.make_async_copy(
            out_h.at[0, :, pl.ds(k * 128, 128)], cur.at[_rows(_arow(k, g), S)], sem.at[1]) for k in range(3)]

    def unit_mm(u, rp, kh):
        xo, wo = _fields(u)[:2]
        ks = range(kh * G // 2, (kh + 1) * G // 2)
        lhs = jnp.concatenate([a[pl.ds(xo + k * S + rp * PR, PR), :] for k in ks], axis=1)
        return jnp.dot(lhs, w[pl.ds(wo + ks[0] * 128, D // 2), :], preferred_element_type=F32)

    def unit(fields, direct=False):
        xo, wo, r0, r1, zo, tr, act = fields
        static = isinstance(act, int)
        lhs = jnp.concatenate([a[_rows(xo + k * S, HB), :] for k in range(G)], axis=1)
        y = jnp.dot(lhs, w[_rows(wo, D), :], preferred_element_type=F32)
        if static:
            if act == 1:
                y = y * QSCALE
            elif act == 2:
                y = _phi(y)
        else:
            y = jnp.where(act == 2, _phi(y), y * jnp.where(act == 1, QSCALE, 1.0))
        if not static or (isinstance(zo, int) and zo < G * 8):
            zacc[_rows(zo, 8), :] += y.reshape(HB // 8, 8, 128).sum(axis=0)
        y_t = jnp.concatenate([y[t * 128:(t + 1) * 128, :].T for t in range(HB // 128)], axis=0)
        if static:
            out = (y_t if tr else y).astype(BF)
        else:
            out = jnp.where(tr == 1, y_t, y).astype(BF)
        dst = cur if direct else a
        dst[_rows(r0, 128), :] = out[:128]
        dst[_rows(r1, 128), :] = out[128:]

    def up_unit(k, r, g=0):
        unit(_fields((k, r, g)), direct=True)

    ctab.start()
    start(d1)
    start(d2)
    start(d3)
    start(cw1)
    zacc[...] = jnp.zeros_like(zacc)
    oacc[...] = jnp.zeros_like(oacc)
    lbuf[...] = jnp.ones_like(lbuf)

    def up_body(n, c):
        @pl.when(n == 1)
        def _():
            wait(cw1)

        @pl.when(n == 2)
        def _():
            wait(dx[1])

        for k in (1, 2, 0):
            for hh in range(TQ // HB):
                up_unit(k, lax.shift_right_logical(n, 1) * (TQ // HB) + hh, n & 1)
        return c
    ctab.wait()
    wait(d1)
    start(dx[1])
    up_unit(1, 0)
    wait(d2)
    start(dx[2])
    up_unit(2, 0)
    up_unit(0, 0)
    wait(d3)
    start(dx[3])
    for k in (1, 2, 0):
        up_unit(k, 1)
    lax.fori_loop(1, 4, up_body, 0)

    eu = SCHED[NB]

    def epi_copy(k):
        return out_copy(eu[k][0], eu[k][2], eu[k][1] * HB, HB)

    part = {}
    npc = 2 * HB // PR

    def piece(n):
        k, rp, kh = n // npc, (n % npc) // 2, n % 2
        y = unit_mm(eu[k], rp, kh)
        if kh == 0:
            part[0] = y
        else:
            a[pl.ds(_fields(eu[k])[2] + rp * PR, PR), :] = (y + part[0]).astype(BF)
        if n % npc == npc - 1:
            epi_copy(k).start()

    def b_mid():
        rr = lax.broadcasted_iota(jnp.int32, (128, 128), 0) // DH
        cc = lax.broadcasted_iota(jnp.int32, (128, 128), 1) // DH
        bd = rr == cc
        zr = lax.broadcasted_iota(jnp.int32, (16, 128), 0)
        zc = lax.broadcasted_iota(jnp.int32, (16, 128), 1) // DH
        kvs = {}

        def kv_half(g, h):
            cs = range(h * G // 2, (h + 1) * G // 2)
            kx = jnp.concatenate(
                [a[pl.ds(_arow(4, c, g * 128), 128), :].astype(F32)
                 + a[pl.ds(_arow(4, c, D + g * 128), 128), :].astype(F32) for c in cs], axis=1)
            return jnp.dot(kx.astype(BF), w[pl.ds(_wrow(4, g, cs[0] * 128), D // 2), :],
                           preferred_element_type=F32)

        def m_half(g, h):
            cs = range(h * G // 2, (h + 1) * G // 2)
            wo = jnp.concatenate([w[pl.ds(_wrow(6, c, g * 128), 128), :] for c in cs], axis=1)
            m = jnp.dot(kvs[g], wo, preferred_element_type=F32).astype(BF)
            for n, c in enumerate(cs):
                w[pl.ds(_wrow(6, c, g * 128), 128), :] = m[:, n * 128:(n + 1) * 128]

        def norm(g, r, z16):
            pq = jnp.concatenate(
                [a[pl.ds(_arow(5, g, (r * TPQ + t) * 128), 128), :] for t in range(TPQ)], axis=1)
            den = jnp.dot(z16, pq, preferred_element_type=F32)
            inv = 1.0 / (den[0:8, :] + 1e-6)
            pqf = pq.astype(F32)
            o_t = jnp.concatenate(
                [pqf[j * DH:(j + 1) * DH, :] * inv[j:j + 1, :] for j in range(4)], axis=0)
            a[pl.ds(_arow(O_B, g, r * TQ), TQ), :] = o_t.T.astype(BF)

        for g in range(G + 1):
            if g < G:
                z = jnp.sum(zacc[g * 8:(g + 1) * 8, :], axis=0, keepdims=True)
                z16 = jnp.where(zr == zc, z, 0.0).astype(BF)
                kv = kv_half(g, 0)
                norm(g, 0, z16)
                kv = kv_half(g, 1) + kv
                kvs[g] = jnp.where(bd, kv, 0.0).astype(BF)
                norm(g, 1, z16)
            for h in range(2):
                if g > 0:
                    m_half(g - 1, h)
                if g < G:
                    norm(g, 2 + h, z16)
                    for n in range((2 * g + h) * NMID * npc // (2 * G), (2 * g + h + 1) * NMID * npc // (2 * G)):
                        piece(n)

    def o_store(o0):
        o_t = jnp.concatenate(
            [oacc[j] * (1.0 / jnp.sum(lbuf[j], axis=0, keepdims=True)) for j in range(4)], axis=0)
        a[_rows(o0, TQ), :] = o_t.T.astype(BF)

    def stage(k0, q0, v0, j, hook):
        sb = sbuf.at[j]
        if k0 is not None:
            qh = jnp.concatenate([cur[_rows(q0 + j * DH + t * 128, DH), :] for t in range(TPQ)], axis=1)
            zero = jnp.zeros((DH, TQ), BF)
            wq = jnp.concatenate([qh if jj == j else zero for jj in range(4)], axis=0)
        if v0 is not None:
            m_prev = jnp.max(mbuf[j], axis=0, keepdims=True)
        m8 = l8 = acc = None
        for c in range(NK):
            rows = slice(c * TK, (c + 1) * TK)
            hook(j, c)

            def qk():
                return jnp.dot(cur[_rows(k0 + c * TK, TK), :], wq, preferred_element_type=F32)
            early = k0 is not None and (j, c) < SLOTS[0]
            if early:
                st = qk()
            if v0 is not None:
                p = jnp.exp2(sb[rows, :] - m_prev)
                for r in reversed(range(TK // 16)):
                    pr = p[r * 16:r * 16 + 8, :] + p[r * 16 + 8:r * 16 + 16, :]
                    l8 = pr if l8 is None else l8 + pr
                o = jnp.dot(cur[_rows(v0 + j * DH + c * TK, DH), :], p.astype(BF), preferred_element_type=F32)
                acc = o if acc is None else o + acc
            if k0 is not None:
                if not early:
                    st = qk()
                sb[rows, :] = st
                mc = st.reshape(TK // 8, 8, TQ).max(axis=0)
                m8 = mc if m8 is None else jnp.maximum(m8, mc)
        if v0 is not None:
            lbuf[j] = l8
            oacc[j] = acc
        if k0 is not None:
            mbuf[j] = m8

    def make_hook(units, slots, o0=None, extra=None):
        def hook(j, c):
            if (j, c) == (0, 2) and extra is not None:
                extra()
            for k, pos in enumerate(slots):
                if pos == (j, c):
                    units[k]()
            if (j, c) == (0, 0) and o0 is not None:
                o_store(o0)
        return hook

    wait(dx[2])
    wait(dx[3])
    start(cw2)
    hook = make_hook([lambda u=u: unit(_fields(u), direct=True) for u in SCHED[0]], SLOTS_0)
    k0, q0 = _body_fields(0)[:2]
    for j in range(4):
        stage(k0, q0, None, j, hook)
        if j == 2:
            start(cw3)
    wait(cw2)

    def body(i, carry):
        ph, g, act = carry
        t0 = i * (NU * NF)
        k0, q0, v0, o0 = (tab[TB0 + i * NBF + n] for n in range(4))
        hook = make_hook([lambda k=k: unit(tuple(tab[t0 + k * NF + n] for n in range(NF))) for k in range(NU)],
                         SLOTS, o0, lambda: pl.when(act == 2)(lambda: start(f_in(g + 1))))

        @pl.when(act == 1)
        def _():
            wait(f_in(g))

        @pl.when(act == 2)
        def _():
            wait(f_out(g + 1))

        for j in range(4):
            stage(k0, q0, v0, j, hook)

        @pl.when(jnp.logical_and(g < G - 1, ph == 0))
        def _():
            start(f_out(g + 1))

        @pl.when(i > MID)
        def _():
            start(late_copies(i - MID - 1))

        @pl.when(jnp.logical_or(i == 3, i == MID))
        def _():
            @pl.when(i == 3)
            def _():
                wait(cw3)

            @pl.when(i == MID)
            def _():
                b_mid()
        wrap = ph == P1 - 1
        act = jnp.where(jnp.logical_and(g >= 1, g < G - 1), jnp.where(wrap, 1, jnp.where(ph == 1, 2, 0)), 0)
        return jnp.where(wrap, 0, ph + 1), jnp.where(wrap, g + 1, g), act
    lax.fori_loop(1, NB, body, (jnp.int32(1), jnp.int32(0), jnp.int32(0)))

    def hook(j, c):
        n = j * NK + c
        for m in range(n * EPI_FINE * npc // (4 * NK), (n + 1) * EPI_FINE * npc // (4 * NK)):
            piece(NMID * npc + m)

    _, _, v0, o0 = _body_fields(NB)
    o_store(o0)
    for j in range(4):
        stage(None, None, v0, j, hook)
    o_store(_body_fields(NB + 1)[3])
    for k in range(NMID + EPI_FINE, NU_EPI):
        unit(_fields(eu[k]))
        epi_copy(k).start()

    for c in range(G - 1):
        wait(late_copies(c))
    for k in range(NU_EPI):
        epi_copy(k).wait()


@jax.jit
def pallas_concat_heads__mha_block__linear_attn_block__prompt_kernel(A_x, A_wqkv, A_wo, B_x, B_wqkv, B_wo):
    any_spec = pl.BlockSpec(memory_space=pl.ANY)
    return pl.pallas_call(
        _kernel,
        out_shape=jax.ShapeDtypeStruct((1, S, 2 * D), BF),
        in_specs=[any_spec] * 7,
        out_specs=any_spec,
        scratch_shapes=[
            pltpu.VMEM((12 * G * S, 128), BF),
            pltpu.VMEM((10 * G * D, 128), BF),
            pltpu.VMEM((3 * G * S, 128), BF),
            pltpu.VMEM((2 * G * 8, 128), F32),
            pltpu.VMEM((4, S, TQ), F32),
            pltpu.VMEM((4, 8, TQ), F32),
            pltpu.VMEM((4, 8, TQ), F32),
            pltpu.VMEM((4, DH, TQ), F32),
            pltpu.SMEM((TAB_LEN,), jnp.int32),
            pltpu.SemaphoreType.DMA((5,)),
        ],
        compiler_params=pltpu.CompilerParams(vmem_limit_bytes=120 * 1024 * 1024, disable_bounds_checks=True),
    )(A_x, A_wqkv, A_wo, B_x, B_wqkv, B_wo, jnp.asarray(_table()))
```

```python
import math
import jax
import jax.numpy as jnp
from jax import lax
import jax.experimental.pallas as pl
import jax.experimental.pallas.tpu as pltpu

S, D, H, DH = 2048, 1024, 32, 32
G = D // 128
TQ = 512
TK = 128
NQ = S // TQ
NK = S // TK
TPQ = TQ // 128
NB = NQ * G
HB = 256
NHB = S // HB
NU = 14
NU_0 = 24
NU_EPI = 30
MID = 24
QSCALE = (DH ** -0.5) * math.log2(math.e)
BF = jnp.bfloat16
F32 = jnp.float32

X_A, X_B, O_B, O_A = 8, 9, 10, 11
U_SRC = (X_A, X_A, X_A, X_B, 3, X_B, O_B, O_A)
U_TR = (0, 1, 1, 1, 0, 1, 0, 0)
U_ACT = (0, 1, 0, 2, 0, 2, 0, 0)
SLOTS = [(j, c) for j in range(4) for c in (3, 7, 11, 15)][:NU]
SLOTS_0 = ([(0, c) for c in (1, 2, 3, 4)] + [(j, c) for j in range(4) for c in range(2, NK, 2)][2:])[:NU_0]
PR = 64
EPI_FINE = 8
NMID = 4
NF = 7
NBF = 4
P1 = 3
ORDER = [(g, q) for g in range(G) for q in range(P1)] + [(g, NQ - 1) for g in range(G)]
RA = P1 * TQ // HB


def _schedule():
    a_units = ([(k, r, g) for g in (0, 1) for k in (0, 2, 1) for r in range(NHB // 2, NHB)]
               + [(k, r, g) for g in range(2, G) for k in (0, 1, 2) for r in range(NHB)])
    b_pre = [(k, r, c) for k in (3, 5, 4) for r in range(NHB) for c in range(G)]

    def late(c):
        return [(6, r, c) for r in range(NHB)] + [(7, r, c) for r in range(RA)]

    sched = [[a_units.pop(0) for _ in range(NU_0)]]
    for i in range(1, MID + 1):
        na = min(len(a_units), 8)
        sched.append([a_units.pop(0) for _ in range(na)] + [b_pre.pop(0) for _ in range(NU - na)])
    assert not a_units and not b_pre
    assert all(k < 3 and c <= 1 for k, r, c in sched[0])
    for i in range(MID + 1, NB):
        sched.append(late(i - MID - 1))
    last = late(G - 1)
    last = last[NHB:NHB + NMID] + last[:NHB] + last[NHB + NMID:]
    sched.append(last + [(7, r, c) for r in range(RA, NHB) for c in range(G)])
    assert all(ORDER.index((g, r // 2)) + 2 <= MID for k, r, c in last[:NMID] for g in range(G))
    assert all(len(us) == NU for us in sched[1:NB]) and len(sched[NB]) == NU_EPI
    done = set((k, r, g) for k in range(3) for r in range(NHB // 2) for g in (0, 1))
    for i in range(NB):
        for k, r, c in sched[i]:
            if k == 4:
                assert all((3, rr, cc) in done for rr in range(NHB) for cc in range(G))
            if k == 7:
                assert all(ORDER.index((g, r // 2)) + 2 <= i for g in range(G)), (i, r)
        assert i > 3 or all(c <= 2 if k < 3 else k == 3 for k, r, c in sched[i])
        done.update(sched[i])
        g = i // P1 + 1
        if g < G and i % P1 == 0:
            assert all((k, r, g) in done for k in (0, 1, 2) for r in range(NHB)), i
    return sched


SCHED = _schedule()


def _arow(slot, tile, row=0):
    return (slot * G + tile) * S + row


def _wrow(slot, tile, row=0):
    return (slot * G + tile) * D + row


def _fields(u):
    k, r, c = u
    wslot = 8 + r // (NHB // 2) if k == 4 else k
    if k == 3:
        dst = [_arow(3, t % G, (t // G) * D + c * 128) for t in (2 * r, 2 * r + 1)]
    else:
        dst = [_arow(k, c, r * HB), _arow(k, c, r * HB + 128)]
    return (_arow(U_SRC[k], 0, r * HB), _wrow(wslot, c), dst[0], dst[1],
            ((0 if k == 3 else G) + c) * 8, U_TR[k], U_ACT[k])


def _body_fields(i):
    g, q = ORDER[min(i, NB - 1)]
    g1 = ORDER[min(max(i - 1, 0), NB - 1)][0]
    g2, q2 = ORDER[max(i - 2, 0)]
    return _arow(0, g), _arow(1, g, q * TQ), _arow(2, g1), _arow(O_A, g2, q2 * TQ)


TB0 = NB * NU * NF
TAB_LEN = TB0 + NB * NBF


def _table():
    t = {}
    for i in range(1, NB):
        for k, u in enumerate(SCHED[i]):
            for n, v in enumerate(_fields(u)):
                t[(i * NU + k) * NF + n] = v
        for n, v in enumerate(_body_fields(i)):
            t[TB0 + i * NBF + n] = v
    return t


def _phi(t):
    return jnp.where(t > 0, t + 1.0, jnp.exp(t)) + 1e-6


def _rows(start, size, align=None):
    if isinstance(start, int):
        return pl.ds(start, size)
    return pl.ds(pl.multiple_of(start, align or size), size)


def _kernel(xa_h, wa_h, woa_h, xb_h, wb_h, wob_h, out_h,
            a, w, cur, zacc, sbuf, mbuf, lbuf, oacc, tab, sem):
    def w_src(slot, c):
        cols = pl.ds(c * 128, 128)
        if slot < 3:
            return wa_h.at[:, pl.ds((1, 0, 2)[slot] * D + c * 128, 128)]
        if slot < 6:
            return wb_h.at[:, pl.ds((1, 2, 0)[slot - 3] * D + c * 128, 128)]
        if slot < 8:
            return (wob_h, woa_h)[slot - 6].at[:, cols]
        return xb_h.at[0, pl.ds((slot - 8) * D, D), cols]

    def cw(pairs, s):
        return [pltpu.make_async_copy(w_src(sl, c), w.at[pl.ds(_wrow(sl, c), D)], sem.at[s]) for sl, c in pairs]

    def cx(src, slot, row, n, s):
        return [pltpu.make_async_copy(src.at[0, pl.ds(row, n), pl.ds(k * 128, 128)],
                                      a.at[pl.ds(_arow(slot, k, row), n)], sem.at[s]) for k in range(G)]

    d1 = cw([(1, 0)], 0) + cx(xa_h, X_A, 0, HB, 0)
    d2 = cw([(2, 0), (0, 0)], 1)
    d3 = cx(xa_h, X_A, HB, HB, 2)
    cw1 = cw([(sl, 1) for sl in (0, 1, 2)], 3)
    dx = [None] + [cx(xa_h, X_A, r * TQ, TQ, r - 1) for r in range(1, NQ)]
    cw2 = cx(xb_h, X_B, 0, S, 3) + cw([(sl, 2) for sl in (0, 1, 2)] + [(3, c) for c in range(G)], 3)
    cw3 = cw([(sl, c) for c in range(3, G) for sl in (0, 1, 2)]
             + [(sl, c) for sl in (5, 8, 9, 4, 6, 7) for c in range(G)], 4)

    def start(cs):
        for c in cs:
            c.start()

    def wait(cs):
        for c in cs:
            c.wait()

    def out_copy(k, c, row, n):
        return pltpu.make_async_copy(
            a.at[_rows(_arow(k, c, row), n, HB)],
            out_h.at[0, pl.ds(row, n), _rows((D if k == 6 else 0) + c * 128, 128)], sem.at[2])

    def late_copies(c):
        return [out_copy(6, c, 0, S), out_copy(7, c, 0, RA * HB)]

    def f_out(g):
        return [pltpu.make_async_copy(
            a.at[_rows(_arow(k, g), S)], out_h.at[0, :, pl.ds(k * 128, 128)], sem.at[0]) for k in range(3)]

    def f_in(g):
        return [pltpu.make_async_copy(
            out_h.at[0, :, pl.ds(k * 128, 128)], cur.at[_rows(_arow(k, g), S)], sem.at[1]) for k in range(3)]

    def unit_mm(u, rp, kh):
        xo, wo = _fields(u)[:2]
        ks = range(kh * G // 2, (kh + 1) * G // 2)
        lhs = jnp.concatenate([a[pl.ds(xo + k * S + rp * PR, PR), :] for k in ks], axis=1)
        return jnp.dot(lhs, w[pl.ds(wo + ks[0] * 128, D // 2), :], preferred_element_type=F32)

    def unit(fields, direct=False):
        xo, wo, r0, r1, zo, tr, act = fields
        static = isinstance(act, int)
        lhs = jnp.concatenate([a[_rows(xo + k * S, HB), :] for k in range(G)], axis=1)
        y = jnp.dot(lhs, w[_rows(wo, D), :], preferred_element_type=F32)
        if static:
            if act == 1:
                y = y * QSCALE
            elif act == 2:
                y = _phi(y)
        else:
            y = jnp.where(act == 2, _phi(y), y * jnp.where(act == 1, QSCALE, 1.0))
        if not static or (isinstance(zo, int) and zo < G * 8):
            zacc[_rows(zo, 8), :] += y.reshape(HB // 8, 8, 128).sum(axis=0)
        y_t = jnp.concatenate([y[t * 128:(t + 1) * 128, :].T for t in range(HB // 128)], axis=0)
        if static:
            out = (y_t if tr else y).astype(BF)
        else:
            out = jnp.where(tr == 1, y_t, y).astype(BF)
        dst = cur if direct else a
        dst[_rows(r0, 128), :] = out[:128]
        dst[_rows(r1, 128), :] = out[128:]

    def up_unit(k, r, g=0):
        unit(_fields((k, r, g)), direct=True)

    start(d1)
    start(d2)
    start(d3)
    start(cw1)
    zacc[...] = jnp.zeros_like(zacc)
    oacc[...] = jnp.zeros_like(oacc)
    lbuf[...] = jnp.ones_like(lbuf)

    def up_body(n, c):
        @pl.when(n == 1)
        def _():
            wait(cw1)

        @pl.when(n == 2)
        def _():
            wait(dx[1])

        for k in (1, 2, 0):
            for hh in range(TQ // HB):
                up_unit(k, lax.shift_right_logical(n, 1) * (TQ // HB) + hh, n & 1)
        return c
    wait(d1)
    start(dx[1])
    up_unit(1, 0)
    wait(d2)
    start(dx[2])
    up_unit(2, 0)
    up_unit(0, 0)
    wait(d3)
    start(dx[3])
    for k in (1, 2, 0):
        up_unit(k, 1)
    lax.fori_loop(1, 4, up_body, 0)

    eu = SCHED[NB]

    def epi_copy(k):
        return out_copy(eu[k][0], eu[k][2], eu[k][1] * HB, HB)

    part = {}
    npc = 2 * HB // PR

    def piece(n):
        k, rp, kh = n // npc, (n % npc) // 2, n % 2
        y = unit_mm(eu[k], rp, kh)
        if kh == 0:
            part[0] = y
        else:
            a[pl.ds(_fields(eu[k])[2] + rp * PR, PR), :] = (y + part[0]).astype(BF)
        if n % npc == npc - 1:
            epi_copy(k).start()

    def b_mid():
        rr = lax.broadcasted_iota(jnp.int32, (128, 128), 0) // DH
        cc = lax.broadcasted_iota(jnp.int32, (128, 128), 1) // DH
        bd = rr == cc
        zr = lax.broadcasted_iota(jnp.int32, (16, 128), 0)
        zc = lax.broadcasted_iota(jnp.int32, (16, 128), 1) // DH
        kvs = {}

        def kv_half(g, h):
            cs = range(h * G // 2, (h + 1) * G // 2)
            kx = jnp.concatenate(
                [a[pl.ds(_arow(4, c, g * 128), 128), :].astype(F32)
                 + a[pl.ds(_arow(4, c, D + g * 128), 128), :].astype(F32) for c in cs], axis=1)
            return jnp.dot(kx.astype(BF), w[pl.ds(_wrow(4, g, cs[0] * 128), D // 2), :],
                           preferred_element_type=F32)

        def m_half(g, h):
            cs = range(h * G // 2, (h + 1) * G // 2)
            wo = jnp.concatenate([w[pl.ds(_wrow(6, c, g * 128), 128), :] for c in cs], axis=1)
            m = jnp.dot(kvs[g], wo, preferred_element_type=F32).astype(BF)
            for n, c in enumerate(cs):
                w[pl.ds(_wrow(6, c, g * 128), 128), :] = m[:, n * 128:(n + 1) * 128]

        def norm(g, r, z16):
            pq = jnp.concatenate(
                [a[pl.ds(_arow(5, g, (r * TPQ + t) * 128), 128), :] for t in range(TPQ)], axis=1)
            den = jnp.dot(z16, pq, preferred_element_type=F32)
            inv = 1.0 / (den[0:8, :] + 1e-6)
            pqf = pq.astype(F32)
            o_t = jnp.concatenate(
                [pqf[j * DH:(j + 1) * DH, :] * inv[j:j + 1, :] for j in range(4)], axis=0)
            a[pl.ds(_arow(O_B, g, r * TQ), TQ), :] = o_t.T.astype(BF)

        for g in range(G + 1):
            if g < G:
                z = jnp.sum(zacc[g * 8:(g + 1) * 8, :], axis=0, keepdims=True)
                z16 = jnp.where(zr == zc, z, 0.0).astype(BF)
                kv = kv_half(g, 0)
                norm(g, 0, z16)
                kv = kv_half(g, 1) + kv
                kvs[g] = jnp.where(bd, kv, 0.0).astype(BF)
                norm(g, 1, z16)
            for h in range(2):
                if g > 0:
                    m_half(g - 1, h)
                if g < G:
                    norm(g, 2 + h, z16)
                    for n in range((2 * g + h) * NMID * npc // (2 * G), (2 * g + h + 1) * NMID * npc // (2 * G)):
                        piece(n)

    def o_store(o0):
        o_t = jnp.concatenate(
            [oacc[j] * (1.0 / jnp.sum(lbuf[j], axis=0, keepdims=True)) for j in range(4)], axis=0)
        a[_rows(o0, TQ), :] = o_t.T.astype(BF)

    def stage(k0, q0, v0, j, hook):
        sb = sbuf.at[j]
        if k0 is not None:
            qh = jnp.concatenate([cur[_rows(q0 + j * DH + t * 128, DH), :] for t in range(TPQ)], axis=1)
            zero = jnp.zeros((DH, TQ), BF)
            wq = jnp.concatenate([qh if jj == j else zero for jj in range(4)], axis=0)
        if v0 is not None:
            m_prev = jnp.max(mbuf[j], axis=0, keepdims=True)
        m8 = l8 = acc = None
        for c in range(NK):
            rows = slice(c * TK, (c + 1) * TK)
            hook(j, c)

            def qk():
                return jnp.dot(cur[_rows(k0 + c * TK, TK), :], wq, preferred_element_type=F32)
            early = k0 is not None and (j, c) < SLOTS[0]
            if early:
                st = qk()
            if v0 is not None:
                p = jnp.exp2(sb[rows, :] - m_prev)
                for r in reversed(range(TK // 16)):
                    pr = p[r * 16:r * 16 + 8, :] + p[r * 16 + 8:r * 16 + 16, :]
                    l8 = pr if l8 is None else l8 + pr
                o = jnp.dot(cur[_rows(v0 + j * DH + c * TK, DH), :], p.astype(BF), preferred_element_type=F32)
                acc = o if acc is None else o + acc
            if k0 is not None:
                if not early:
                    st = qk()
                sb[rows, :] = st
                mc = st.reshape(TK // 8, 8, TQ).max(axis=0)
                m8 = mc if m8 is None else jnp.maximum(m8, mc)
        if v0 is not None:
            lbuf[j] = l8
            oacc[j] = acc
        if k0 is not None:
            mbuf[j] = m8

    def make_hook(units, slots, o0=None, extra=None):
        def hook(j, c):
            if (j, c) == (0, 2) and extra is not None:
                extra()
            for k, pos in enumerate(slots):
                if pos == (j, c):
                    units[k]()
            if (j, c) == (0, 0) and o0 is not None:
                o_store(o0)
        return hook

    start(cw2)
    wait(dx[2])
    wait(dx[3])
    for n, v in _table().items():
        tab[n] = v
    hook = make_hook([lambda u=u: unit(_fields(u), direct=True) for u in SCHED[0]], SLOTS_0)
    k0, q0 = _body_fields(0)[:2]
    for j in range(4):
        stage(k0, q0, None, j, hook)
        if j == 2:
            start(cw3)
    wait(cw2)

    def body(i, carry):
        ph, g, act = carry
        t0 = i * (NU * NF)
        k0, q0, v0, o0 = (tab[TB0 + i * NBF + n] for n in range(4))
        hook = make_hook([lambda k=k: unit(tuple(tab[t0 + k * NF + n] for n in range(NF))) for k in range(NU)],
                         SLOTS, o0, lambda: pl.when(act == 2)(lambda: start(f_in(g + 1))))

        @pl.when(act == 1)
        def _():
            wait(f_in(g))

        @pl.when(act == 2)
        def _():
            wait(f_out(g + 1))

        for j in range(4):
            stage(k0, q0, v0, j, hook)

        @pl.when(jnp.logical_and(g < G - 1, ph == 0))
        def _():
            start(f_out(g + 1))

        @pl.when(i > MID)
        def _():
            start(late_copies(i - MID - 1))

        @pl.when(jnp.logical_or(i == 3, i == MID))
        def _():
            @pl.when(i == 3)
            def _():
                wait(cw3)

            @pl.when(i == MID)
            def _():
                b_mid()
        wrap = ph == P1 - 1
        act = jnp.where(jnp.logical_and(g >= 1, g < G - 1), jnp.where(wrap, 1, jnp.where(ph == 1, 2, 0)), 0)
        return jnp.where(wrap, 0, ph + 1), jnp.where(wrap, g + 1, g), act
    lax.fori_loop(1, NB, body, (jnp.int32(1), jnp.int32(0), jnp.int32(0)))

    def hook(j, c):
        n = j * NK + c
        for m in range(n * EPI_FINE * npc // (4 * NK), (n + 1) * EPI_FINE * npc // (4 * NK)):
            piece(NMID * npc + m)

    _, _, v0, o0 = _body_fields(NB)
    o_store(o0)
    for j in range(4):
        stage(None, None, v0, j, hook)
    o_store(_body_fields(NB + 1)[3])
    for k in range(NMID + EPI_FINE, NU_EPI):
        unit(_fields(eu[k]))
        epi_copy(k).start()

    for c in range(G - 1):
        wait(late_copies(c))
    for k in range(NU_EPI):
        epi_copy(k).wait()


@jax.jit
def pallas_concat_heads__mha_block__linear_attn_block__prompt_kernel(A_x, A_wqkv, A_wo, B_x, B_wqkv, B_wo):
    any_spec = pl.BlockSpec(memory_space=pl.ANY)
    return pl.pallas_call(
        _kernel,
        out_shape=jax.ShapeDtypeStruct((1, S, 2 * D), BF),
        in_specs=[any_spec] * 6,
        out_specs=any_spec,
        scratch_shapes=[
            pltpu.VMEM((12 * G * S, 128), BF),
            pltpu.VMEM((10 * G * D, 128), BF),
            pltpu.VMEM((3 * G * S, 128), BF),
            pltpu.VMEM((2 * G * 8, 128), F32),
            pltpu.VMEM((4, S, TQ), F32),
            pltpu.VMEM((4, 8, TQ), F32),
            pltpu.VMEM((4, 8, TQ), F32),
            pltpu.VMEM((4, DH, TQ), F32),
            pltpu.SMEM((TAB_LEN,), jnp.int32),
            pltpu.SemaphoreType.DMA((5,)),
        ],
        compiler_params=pltpu.CompilerParams(vmem_limit_bytes=120 * 1024 * 1024, disable_bounds_checks=True),
    )(A_x, A_wqkv, A_wo, B_x, B_wqkv, B_wo)
```
